```python
import os as _os
_os.environ.setdefault("JAX_PLATFORMS", "cpu")
import jax
import jax.numpy as jnp

def _softmax(x, axis=-1):
    return jax.nn.softmax(x, axis=axis)
def _gelu(x):
    return jax.nn.gelu(x, approximate=True)
def _silu(x):
    return jax.nn.silu(x)
def _sigmoid(x):
    return jax.nn.sigmoid(x)
def _layernorm(x, axis=-1, eps=1e-5):
    m = jnp.mean(x, axis=axis, keepdims=True)
    v = jnp.var(x, axis=axis, keepdims=True)
    return (x - m) / jnp.sqrt(v + eps)
def _scatter_add(tgt, idx, src, axis=0):
    return tgt.at[idx].add(src)
def _segment_sum(src, seg, n):
    return jax.ops.segment_sum(src, seg, n)
class _Rng:
    def __init__(self, key):
        self._k = key
    def _next(self):
        self._k, sub = jax.random.split(self._k)
        return sub
    def normal(self, shape):
        return jax.random.normal(self._next(), shape, dtype=jnp.bfloat16)
    def randint(self, lo, hi, shape):
        return jax.random.randint(self._next(), shape, lo, hi, dtype=jnp.int32)
    def uniform(self, shape, lo=0.0, hi=1.0):
        return jax.random.uniform(self._next(), shape, jnp.bfloat16, lo, hi)
    def permutation(self, n):
        return jax.random.permutation(self._next(), n)


kernel_name = 'concat_heads__gqa_block_cached__mha_block_cached__near_ridge'

def setup_inputs():
    _rng = _Rng(jax.random.key(int.from_bytes(__import__("os").urandom(4), "little")))
    _w = (lambda a: (lambda t: t.astype(jnp.bfloat16) if jnp.issubdtype(t.dtype, jnp.floating) else t)(jnp.asarray(a)))
    def _A_setup():
        B, Sq, D = 8, 112, 448
        Hq, Hkv, Sk, Dh = 16, 8, 512, 256
        assert Hq % Hkv == 0, (Hq, Hkv)
        return {
            "x": _w((lambda *s: _rng.normal(s) * 0.8)(B, Sq, D)),
            "k_cache": _w((lambda *s: _rng.normal(s) * 0.8)(B, Hkv, Sk, Dh)),
            "v_cache": _w((lambda *s: _rng.normal(s) * 0.05)(B, Hkv, Sk, Dh)),
            "wq": _w((lambda *s: _rng.normal(s) * 0.8)(D, Hq * Dh) * (D ** -0.5)),
            "wo": _w((lambda *s: _rng.normal(s) * 0.05)(Hq * Dh, D) * ((Hq * Dh) ** -0.5)),
        }
    _A_in = _A_setup()

    def _B_setup():
        B, Sq, D = 8, 112, 448
        H, Sk, Dh = 16, 512, 256
        return {
            "x": _w((lambda *s: _rng.normal(s) * 0.8)(B, Sq, D)),
            "k_cache": _w((lambda *s: _rng.normal(s) * 0.8)(B, H, Sk, Dh)),
            "v_cache": _w((lambda *s: _rng.normal(s) * 0.05)(B, H, Sk, Dh)),
            "wq": _w((lambda *s: _rng.normal(s) * 0.8)(D, H * Dh) * (D ** -0.5)),
            "wo": _w((lambda *s: _rng.normal(s) * 0.05)(H * Dh, D) * ((H * Dh) ** -0.5)),
        }
    _B_in = _B_setup()

    return {
        "A_x": _A_in["x"],
        "A_k_cache": _A_in["k_cache"],
        "A_v_cache": _A_in["v_cache"],
        "A_wq": _A_in["wq"],
        "A_wo": _A_in["wo"],
        "B_x": _B_in["x"],
        "B_k_cache": _B_in["k_cache"],
        "B_v_cache": _B_in["v_cache"],
        "B_wq": _B_in["wq"],
        "B_wo": _B_in["wo"],
    }

def reference(A_x, A_k_cache, A_v_cache, A_wq, A_wo, B_x, B_k_cache, B_v_cache, B_wq, B_wo):
    def _A_ref(x, k_cache, v_cache, wq, wo):
        B, Sq, D = x.shape
        Hq, Dh = 16, 256
        Hkv = k_cache.shape[1]
        rep = Hq // Hkv
        q = (lambda x, *d: x.transpose(*d))((x @ wq).reshape(B, Sq, Hq, Dh), 0, 2, 1, 3)
        k = jnp.repeat(k_cache, rep, axis=1)
        v = jnp.repeat(v_cache, rep, axis=1)
        scores = jnp.einsum("bhqd,bhkd->bhqk", q, k) * (Dh ** -0.5)
        p = _softmax(scores, axis=-1)
        o = jnp.einsum("bhqk,bhkd->bhqd", p, v)
        return (lambda x, *d: x.transpose(*d))(o, 0, 2, 1, 3).reshape(B, Sq, Hq * Dh) @ wo

    def _B_ref(x, k_cache, v_cache, wq, wo):
        B, Sq, D = x.shape
        H, Dh = 16, 256
        q = (lambda x, *d: x.transpose(*d))((x @ wq).reshape(B, Sq, H, Dh), 0, 2, 1, 3)
        scores = jnp.einsum("bhqd,bhkd->bhqk", q, k_cache) * (Dh ** -0.5)
        p = _softmax(scores, axis=-1)
        o = jnp.einsum("bhqk,bhkd->bhqd", p, v_cache)
        return (lambda x, *d: x.transpose(*d))(o, 0, 2, 1, 3).reshape(B, Sq, H * Dh) @ wo

    a = _A_ref(A_x, A_k_cache, A_v_cache, A_wq, A_wo)
    b = _B_ref(B_x, B_k_cache, B_v_cache, B_wq, B_wo)
    return jnp.concatenate([a, b], axis=-1)
```

```python
import functools
import math
import jax
import jax.numpy as jnp
from jax import lax
import jax.experimental.pallas as pl
import jax.experimental.pallas.tpu as pltpu

B, SQ, D = 8, 112, 448
H, SK, DH = 16, 512, 256
M = B * SQ
G = 8
GW = 2 * DH
QSCALE = DH ** -0.5 * math.log2(math.e)
NT = (((1,), (1,)), ((), ()))
bf16 = jnp.bfloat16
f32 = jnp.float32
NODMA = False


def _qk(q, k):
    return lax.dot_general(q, k, NT, preferred_element_type=f32)


def _softmax(s):
    m = jnp.max(s, axis=-1, keepdims=True)
    p = jnp.exp2(s - m)
    l = jnp.sum(p, axis=-1, keepdims=True)
    return p.astype(bf16), l


def _pv(p, l, v):
    o = jnp.dot(p, v, preferred_element_type=f32)
    return (o * (1.0 / l)).astype(bf16)


def kernel(xa_h, ka_h, va_h, wqa_h, woa_h, xb_h, kb_h, vb_h, wqb_h, wob_h, out_h,
           x_v, wq_v, wo_v, ka_v, va_v, kb_v, vb_v, q0_s, o_s, acc, out_v,
           x_sem, w_sem, kv_sem, out_sem):
    g = pl.program_id(0)

    def x_copy(i):
        return pltpu.make_async_copy((xa_h, xb_h)[i], x_v.at[i], x_sem.at[i])

    def w_copy(i, gg):
        src = (wqa_h, wqb_h, woa_h, wob_h)[i]
        dst = (wq_v, wq_v, wo_v, wo_v)[i]
        col = pl.ds(pl.multiple_of(gg * GW, GW), GW)
        return pltpu.make_async_copy(src.at[:, col], dst.at[i % 2, :, col], w_sem.at[i, gg % 2])

    def kv_copy(i, gg, b):
        if i < 2:
            src = (ka_h, va_h)[i].at[b, gg]
            dst = (ka_v, va_v)[i].at[b]
        else:
            src = (kb_h, vb_h)[i - 2].at[b, pl.ds(2 * gg, 2)]
            dst = (kb_v, vb_v)[i - 2].at[b]
        return pltpu.make_async_copy(src, dst, kv_sem.at[i, b])

    def start(c):
        if not NODMA:
            c.start()

    def wait(c):
        if not NODMA:
            c.wait()

    def qproj(br, b, gg):
        col = pl.ds(pl.multiple_of(gg * GW, GW), GW)
        q = jnp.dot(x_v[br, b * SQ:(b + 1) * SQ, :], wq_v[br, :, col], preferred_element_type=f32)
        return (q * QSCALE).astype(bf16)

    @pl.when(g == 0)
    def _():
        start(w_copy(0, 0)); start(x_copy(0)); start(kv_copy(0, 0, 0))
        start(w_copy(1, 0)); start(x_copy(1))
        for i in (1, 2, 3):
            start(kv_copy(i, 0, 0))
        for i in range(4):
            start(kv_copy(i, 0, 1))
        start(w_copy(2, 0)); start(w_copy(3, 0))
        for b in range(2, B):
            for i in range(4):
                start(kv_copy(i, 0, b))
        acc[...] = jnp.zeros(acc.shape, f32)
        wait(w_copy(0, 0)); wait(x_copy(0))
        q0_s[0] = qproj(0, 0, 0)
        wait(w_copy(1, 0)); wait(x_copy(1))
        q0_s[1] = qproj(1, 0, 0)

    gcol = pl.ds(pl.multiple_of(g * GW, GW), GW)
    gn = jnp.minimum(g + 1, G - 1)

    @pl.when(g < G - 1)
    def _():
        for i in range(4):
            start(w_copy(i, g + 1))

    def oproj(br, j):
        t = lax.dot_general(wo_v[br, :, gcol], o_s[br, j * 128:(j + 1) * 128, :], NT, preferred_element_type=f32)
        acc[br * D:(br + 1) * D, j * 128:(j + 1) * 128] += t

    def refill(b):
        @pl.when(g < G - 1)
        def _():
            for i in range(4):
                start(kv_copy(i, g + 1, b))

    qa = q0_s[0]
    qb = q0_s[1]
    pend = None
    for b in range(B):
        rows = slice(b * SQ, (b + 1) * SQ)
        for i in range(4):
            wait(kv_copy(i, g, b))
        if b == 2:
            wait(w_copy(2, g)); wait(w_copy(3, g))
        sa = _qk(jnp.concatenate([qa[:, :DH], qa[:, DH:]], axis=0), ka_v[b])
        if pend is not None:
            o_s[1, (b - 1) * SQ:b * SQ, DH:] = _pv(pend[0], pend[1], vb_v[b - 1, 1])
        sb0 = _qk(qb[:, :DH], kb_v[b, 0])
        pa, la = _softmax(sa)
        oa = _pv(pa, la, va_v[b])
        o_s[0, rows, :DH] = oa[:SQ]
        o_s[0, rows, DH:] = oa[SQ:]
        sb1 = _qk(qb[:, DH:], kb_v[b, 1])
        pb0, lb0 = _softmax(sb0)
        o_s[1, rows, :DH] = _pv(pb0, lb0, vb_v[b, 0])
        pend = _softmax(sb1)
        if b < B - 1:
            qa = qproj(0, b + 1, g)
            qb = qproj(1, b + 1, g)
        if b >= 2:
            oproj(0, b - 2)
            oproj(1, b - 2)
        if b >= 1 and not NODMA:
            refill(b - 1)
    if not NODMA:
        @pl.when(g < G - 1)
        def _():
            wait(w_copy(0, g + 1)); wait(w_copy(1, g + 1))
    q0_s[0] = qproj(0, 0, gn)
    o_s[1, (B - 1) * SQ:, DH:] = _pv(pend[0], pend[1], vb_v[B - 1, 1])
    oproj(0, B - 2)
    q0_s[1] = qproj(1, 0, gn)
    oproj(1, B - 2)
    if not NODMA:
        refill(B - 1)

    @pl.when(g == G - 1)
    def _():
        out_v[...] = acc[...].T.astype(bf16)
        c = pltpu.make_async_copy(out_v, out_h, out_sem)
        c.start()
        c.wait()


@jax.jit
def pallas_concat_heads__gqa_block_cached__mha_block_cached__near_ridge_kernel(A_x, A_k_cache, A_v_cache, A_wq, A_wo, B_x, B_k_cache, B_v_cache, B_wq, B_wo):
    xa = A_x.reshape(M, D)
    xb = B_x.reshape(M, D)
    hbm = pl.BlockSpec(memory_space=pltpu.MemorySpace.HBM)
    out = pl.pallas_call(
        kernel,
        grid=(G,),
        in_specs=[hbm] * 10,
        out_specs=hbm,
        out_shape=jax.ShapeDtypeStruct((M, 2 * D), bf16),
        scratch_shapes=[
            pltpu.VMEM((2, M, D), bf16),
            pltpu.VMEM((2, D, H * DH), bf16),
            pltpu.VMEM((2, D, H * DH), bf16),
            pltpu.VMEM((B, SK, DH), bf16),
            pltpu.VMEM((B, SK, DH), bf16),
            pltpu.VMEM((B, 2, SK, DH), bf16),
            pltpu.VMEM((B, 2, SK, DH), bf16),
            pltpu.VMEM((2, SQ, GW), bf16),
            pltpu.VMEM((2, M, GW), bf16),
            pltpu.VMEM((2 * D, M), f32),
            pltpu.VMEM((M, 2 * D), bf16),
            pltpu.SemaphoreType.DMA((2,)),
            pltpu.SemaphoreType.DMA((4, 2)),
            pltpu.SemaphoreType.DMA((4, B)),
            pltpu.SemaphoreType.DMA(()),
        ],
        compiler_params=pltpu.CompilerParams(
            dimension_semantics=("arbitrary",),
            vmem_limit_bytes=100 * 1024 * 1024,
        ),
    )(xa, A_k_cache, A_v_cache, A_wq, A_wo.T, xb, B_k_cache, B_v_cache, B_wq, B_wo.T)
    return out.reshape(B, SQ, 2 * D)
```

```python
import functools
import math
import jax
import jax.numpy as jnp
from jax import lax
import jax.experimental.pallas as pl
import jax.experimental.pallas.tpu as pltpu

B, SQ, D = 8, 112, 448
H, SK, DH = 16, 512, 256
M = B * SQ
G = 8
GW = 2 * DH
QSCALE = DH ** -0.5 * math.log2(math.e)
NT = (((1,), (1,)), ((), ()))
bf16 = jnp.bfloat16
f32 = jnp.float32
QA = 3
MWAITS = (0, 4)
TWAITS = (0, 2, 3, 4, 5, 6, 7)
NSLOT = 2
F5 = 0
ORDER = 1
QFIRST = 1
SPLIT = 0
ROWS = 512


def _qk(q, k):
    return lax.dot_general(q, k, NT, preferred_element_type=f32)


def _softmax(s):
    m = jnp.max(s, axis=-1, keepdims=True)
    p = jnp.exp2(s - m)
    l = jnp.sum(p, axis=-1, keepdims=True)
    return p.astype(bf16), l


def _pv(p, l, v):
    o = jnp.dot(p, v, preferred_element_type=f32)
    r = pl.reciprocal(l, approx=True)
    r = r * (2.0 - l * r)
    return (o * r).astype(bf16)


def kernel(xa_h, ka_h, va_h, wqa_h, woa_h, xb_h, kb_h, vb_h, wqb_h, wob_h, out_h,
           x_v, wq_v, wo_v, kv_v, q_s, o_s, acc, out_v,
           x_sem, wq_sem, wo_sem, kv_sem, out_sem, reg_sem):
    g = pl.program_id(0)

    def cols(gg):
        return pl.ds(pl.multiple_of(gg * GW, GW), GW)

    def x_copy(i):
        return pltpu.make_async_copy((xa_h, xb_h)[i], x_v.at[i], x_sem.at[i])

    def wq_copy(br, gg):
        return pltpu.make_async_copy((wqa_h, wqb_h)[br].at[:, cols(gg)], wq_v.at[br, :, cols(gg)], wq_sem.at[br, gg])

    def wq_wait(br, gg):
        pltpu.make_async_copy(wq_v.at[br, :, cols(gg)], wq_v.at[br, :, cols(gg)], wq_sem.at[br, gg]).wait()

    def wo_copy(br, gg):
        return pltpu.make_async_copy((woa_h, wob_h)[br].at[:, cols(gg)], wo_v.at[br, :, cols(gg)], wo_sem.at[br, gg])

    def kv_start(gg, b):
        s = gg % NSLOT
        sem = kv_sem.at[s, b]
        r = pl.ds(0, ROWS)
        pltpu.make_async_copy(ka_h.at[b, gg, r], kv_v.at[s, b, 0, r], sem).start()
        pltpu.make_async_copy(va_h.at[b, gg, r], kv_v.at[s, b, 1, r], sem).start()
        pltpu.make_async_copy(kb_h.at[b, pl.ds(2 * gg, 2), r], kv_v.at[s, b, pl.ds(2, 2), r], sem).start()
        pltpu.make_async_copy(vb_h.at[b, pl.ds(2 * gg, 2), r], kv_v.at[s, b, pl.ds(4, 2), r], sem).start()

    def kv_wait(gg, b):
        s = gg % NSLOT
        pltpu.make_async_copy(kv_v.at[s, b, :, pl.ds(0, ROWS)], kv_v.at[s, b, :, pl.ds(0, ROWS)], kv_sem.at[s, b]).wait()

    def out_copy(j):
        r = pl.ds(j * 128, 128)
        return pltpu.make_async_copy(out_v.at[r], out_h.at[r], out_sem.at[j])

    def fence():
        pl.semaphore_signal(reg_sem, 1)
        pl.semaphore_wait(reg_sem, 1)

    def qpiece(br, gg, j):
        c = pl.ds(pl.multiple_of(gg * GW + j * 128, 128), 128)
        q = jnp.dot(x_v[br], wq_v[br, :, c], preferred_element_type=f32)
        q = (q * QSCALE).astype(bf16)
        h, half = j // 2, j % 2
        for b in range(B):
            q_s[br, gg, b, h * SQ:(h + 1) * SQ, half * 128:(half + 1) * 128] = q[b * SQ:(b + 1) * SQ]

    @pl.when(g == 0)
    def _():
        wq_copy(0, 0).start(); x_copy(0).start()
        fence()
        wq_copy(1, 0).start(); x_copy(1).start()
        fence()
        for gg in range(1, QA):
            for br in range(2):
                wq_copy(br, gg).start()
        def issue(gg, lo, hi):
            if lo == 0:
                for br in range(2):
                    wo_copy(br, gg).start()
                    wq_copy(br, gg + QA).start()
            for b in range(lo, hi):
                kv_start(gg, b)

        fence()
        issue(0, 0, 4)
        fence()
        issue(0, 4, 8)
        acc[...] = jnp.zeros(acc.shape, f32)

        def qbody(i, c):
            br = i % 2
            gg = i // 2

            @pl.when(i < 2)
            def _():
                pltpu.make_async_copy(x_v.at[br], x_v.at[br], x_sem.at[br]).wait()
            wq_wait(br, gg)

            @pl.when(i == 2)
            def _():
                issue(1, 0, 4)

            @pl.when(i == 4)
            def _():
                issue(1, 4, 8)
            for j in range(4):
                qpiece(br, gg, j)
            return c
        with jax.named_scope('qloop'):
            lax.fori_loop(0, 2 * QA, qbody, 0)

    def group(main):
        waits = MWAITS if main else TWAITS
        slot = g % NSLOT
        kv = kv_v.at[slot]
        gcol = cols(g)
        gn = g + NSLOT

        @pl.when(gn < G)
        def _():
            for br in range(2):
                wo_copy(br, gn).start()

        if main:
            @pl.when(gn + QA < G)
            def _():
                for br in range(2):
                    wq_copy(br, gn + QA).start()

        def oproj(br, j):
            t = lax.dot_general(wo_v[br, :, gcol], o_s[br, j * 128:(j + 1) * 128, :], NT, preferred_element_type=f32)
            acc[br * D:(br + 1) * D, j * 128:(j + 1) * 128] += t

        def finish(j):
            if main:
                return
            out_v[j * 128:(j + 1) * 128, :] = acc[:, j * 128:(j + 1) * 128].T.astype(bf16)

        def refill(b):
            @pl.when(gn < G)
            def _():
                kv_start(gn, b)

        def do_waits(b):
            if b in waits:
                with jax.named_scope('w%d' % b):
                    nxt = min([w for w in waits if w > b] + [B])
                    for bb in range(b, nxt):
                        kv_wait(g, bb)
                    if b == 0:
                        for br in range(2):
                            wo_copy(br, g).wait()
                            if main:
                                wq_wait(br, g + QA)

        def oproj_half(br, j, h):
            c = pl.ds(pl.multiple_of(g * GW + h * DH, DH), DH)
            t = lax.dot_general(wo_v[br, :, c], o_s[br, j * 128:(j + 1) * 128, h * DH:(h + 1) * DH], NT, preferred_element_type=f32)
            acc[br * D:(br + 1) * D, j * 128:(j + 1) * 128] += t

        S = {}
        P = {}

        def qk(c, b):
            if c == 'a':
                S[c, b] = _qk(q_s[0, g, b], kv[b, 0])
            elif c == 'b0':
                S[c, b] = _qk(q_s[1, g, b, :SQ], kv[b, 2])
            else:
                S[c, b] = _qk(q_s[1, g, b, SQ:], kv[b, 3])

        def sm(c, b):
            P[c, b] = _softmax(S.pop((c, b)))

        def pv(c, b):
            if b < 0:
                return
            if (c, b) not in P:
                sm(c, b)
            p, l = P.pop((c, b))
            rows = slice(b * SQ, (b + 1) * SQ)
            if c == 'a':
                oa = _pv(p, l, kv[b, 1])
                o_s[0, rows, :DH] = oa[:SQ]
                o_s[0, rows, DH:] = oa[SQ:]
            elif c == 'b0':
                o_s[1, rows, :DH] = _pv(p, l, kv[b, 4])
            else:
                o_s[1, rows, DH:] = _pv(p, l, kv[b, 5])

        def op(br, j):
            if j >= 0:
                oproj(br, j)

        def out_start(js):
            @pl.when(g == G - 1)
            def _():
                for j in js:
                    out_copy(j).start()

        def attn(b, with_pend=True):
            if ORDER == 0:
                qk('a', b)
                if with_pend:
                    pv('b1', b - 1)
                qk('b0', b); pv('a', b); qk('b1', b); pv('b0', b)
            elif ORDER == 1:
                if with_pend:
                    pv('b1', b - 1)
                qk('a', b); qk('b0', b); pv('a', b); qk('b1', b); pv('b0', b)
            elif ORDER == 2:
                if with_pend:
                    pv('b1', b - 1)
                qk('a', b); qk('b0', b); qk('b1', b); pv('a', b); pv('b0', b)
            sm('b1', b)

        if not main:
            for b in range(B):
                do_waits(b)
                if b == B - 1:
                    out_start(range(B - 2 if F5 else B - 3))
                    fence()
                    if not F5:
                        finish(B - 3)
                        out_start([B - 3])
                elif b >= 3:
                    finish(b - 3)
                attn(b, with_pend=(b < B - 1))
                if b < B - 2:
                    op(0, b - 1)
                    op(1, b - 2)
                    if b >= 1:
                        refill(b - 1)
                elif b == B - 2:
                    op(1, b - 2)
                    finish(b - 2)
                    pv('b1', b)
                    op(0, b - 1)
                    op(1, b - 1)
                    if F5:
                        finish(b - 1)
                    refill(b - 1)
                    refill(b)
                else:
                    if SPLIT:
                        oproj_half(1, b - 1, 0)
                        pv('b1', b)
                        op(0, b - 1)
                        oproj_half(1, b - 1, 1)
                    else:
                        op(0, b - 1)
                        pv('b1', b)
                        op(1, b - 1)
                    refill(b)
            finish(B - 2)
            out_start([B - 2])
            return

        for b in range(B):
            do_waits(b)
            if QFIRST and b in waits:
                qpiece(b // 4, g + QA, b % 4)
            attn(b)
            if b < B - 1 and not (QFIRST and b in waits):
                qpiece(b // 4, g + QA, b % 4)
            op(0, b - 2)
            op(1, b - 2)
            if b >= 1:
                refill(b - 1)
        op(0, B - 2)
        pv('b1', B - 1)
        qpiece(1, g + QA, 3)
        op(1, B - 2)
        refill(B - 1)

    @pl.when(g < G - QA)
    def _():
        with jax.named_scope('main'):
            group(True)

    @pl.when(g >= G - QA)
    def _():
        with jax.named_scope('tail'):
            group(False)

    @pl.when(g == G - 1)
    def _():
        with jax.named_scope('outwait'):
            for j in range(7):
                out_copy(j).wait()


@jax.jit
def pallas_concat_heads__gqa_block_cached__mha_block_cached__near_ridge_kernel(A_x, A_k_cache, A_v_cache, A_wq, A_wo, B_x, B_k_cache, B_v_cache, B_wq, B_wo):
    xa = A_x.reshape(M, D)
    xb = B_x.reshape(M, D)
    hbm = pl.BlockSpec(memory_space=pltpu.MemorySpace.HBM)
    out = pl.pallas_call(
        kernel,
        grid=(G,),
        in_specs=[hbm] * 10,
        out_specs=hbm,
        out_shape=jax.ShapeDtypeStruct((M, 2 * D), bf16),
        scratch_shapes=[
            pltpu.VMEM((2, M, D), bf16),
            pltpu.VMEM((2, D, H * DH), bf16),
            pltpu.VMEM((2, D, H * DH), bf16),
            pltpu.VMEM((NSLOT, B, 6, SK, DH), bf16),
            pltpu.VMEM((2, G, B, 2 * SQ, DH), bf16),
            pltpu.VMEM((2, M, GW), bf16),
            pltpu.VMEM((2 * D, M), f32),
            pltpu.VMEM((M, 2 * D), bf16),
            pltpu.SemaphoreType.DMA((2,)),
            pltpu.SemaphoreType.DMA((2, G)),
            pltpu.SemaphoreType.DMA((2, G)),
            pltpu.SemaphoreType.DMA((NSLOT, B)),
            pltpu.SemaphoreType.DMA((7,)),
            pltpu.SemaphoreType.REGULAR,
        ],
        compiler_params=pltpu.CompilerParams(
            dimension_semantics=("arbitrary",),
            vmem_limit_bytes=100 * 1024 * 1024,
            disable_bounds_checks=True,
            disable_semaphore_checks=True,
        ),
    )(xa, A_k_cache, A_v_cache, A_wq, A_wo.T, xb, B_k_cache, B_v_cache, B_wq, B_wo.T)
    return out.reshape(B, SQ, 2 * D)
```

```python
import functools
import math
import jax
import jax.numpy as jnp
from jax import lax
import jax.experimental.pallas as pl
import jax.experimental.pallas.tpu as pltpu

B, SQ, D = 8, 112, 448
H, SK, DH = 16, 512, 256
M = B * SQ
G = 8
GW = 2 * DH
QSCALE = DH ** -0.5 * math.log2(math.e)
NT = (((1,), (1,)), ((), ()))
bf16 = jnp.bfloat16
f32 = jnp.float32
QA = 3
MWAITS = (0, 4)
TWAITS = (0, 2, 3, 4, 5, 6, 7)
NSLOT = 2
OA1 = 1
GF = 7
WQB4 = 1
LT = 2
LA = 5
PLO = 1
F5 = 0
ORDER = 1
QFIRST = 1
SPLIT = 0
ROWS = 512


def _qk(q, k):
    return lax.dot_general(q, k, NT, preferred_element_type=f32)


def _softmax(s):
    m = jnp.max(s, axis=-1, keepdims=True)
    p = jnp.exp2(s - m)
    l = jnp.sum(p, axis=-1, keepdims=True)
    return p.astype(bf16), l


def _pv(p, l, v):
    o = jnp.dot(p, v, preferred_element_type=f32)
    r = pl.reciprocal(l, approx=True)
    r = r * (2.0 - l * r)
    return (o * r).astype(bf16)


def kernel(xa_h, ka_h, va_h, wqa_h, woa_h, xb_h, kb_h, vb_h, wqb_h, wob_h, out_h,
           x_v, wq_v, wo_v, kv_v, q_s, o_s, acc, out_v,
           x_sem, wq_sem, wo_sem, kv_sem, out_sem, reg_sem):
    g = pl.program_id(0)

    def cols(gg):
        return pl.ds(pl.multiple_of(gg * GW, GW), GW)

    def x_copy(i):
        return pltpu.make_async_copy((xa_h, xb_h)[i], x_v.at[i], x_sem.at[i])

    def wq_copy(br, gg):
        return pltpu.make_async_copy((wqa_h, wqb_h)[br].at[:, cols(gg)], wq_v.at[br, :, cols(gg)], wq_sem.at[br, gg])

    def wq_wait(br, gg):
        pltpu.make_async_copy(wq_v.at[br, :, cols(gg)], wq_v.at[br, :, cols(gg)], wq_sem.at[br, gg]).wait()

    def wo_copy(br, gg):
        return pltpu.make_async_copy((woa_h, wob_h)[br].at[:, cols(gg)], wo_v.at[br, :, cols(gg)], wo_sem.at[br, gg])

    def kva_start(gg, b, prio):
        s = gg % NSLOT
        sem = kv_sem.at[s, b]
        r = pl.ds(0, ROWS)
        pltpu.make_async_copy(ka_h.at[b, gg, r], kv_v.at[s, b, 0, r], sem).start(priority=prio)
        pltpu.make_async_copy(va_h.at[b, gg, r], kv_v.at[s, b, 1, r], sem).start(priority=prio)

    def kvb_start(gg, b):
        s = gg % NSLOT
        sem = kv_sem.at[s, b]
        r = pl.ds(0, ROWS)
        pltpu.make_async_copy(kb_h.at[b, pl.ds(2 * gg, 2), r], kv_v.at[s, b, pl.ds(2, 2), r], sem).start(priority=PLO)
        pltpu.make_async_copy(vb_h.at[b, pl.ds(2 * gg, 2), r], kv_v.at[s, b, pl.ds(4, 2), r], sem).start(priority=PLO)

    def kv_wait(gg, b):
        s = gg % NSLOT
        pltpu.make_async_copy(kv_v.at[s, b, :, pl.ds(0, ROWS)], kv_v.at[s, b, :, pl.ds(0, ROWS)], kv_sem.at[s, b]).wait()

    def out_copy(j):
        r = pl.ds(j * 128, 128)
        return pltpu.make_async_copy(out_v.at[r], out_h.at[r], out_sem.at[j])

    def fence():
        pl.semaphore_signal(reg_sem, 1)
        pl.semaphore_wait(reg_sem, 1)

    def qpiece(br, gg, j):
        c = pl.ds(pl.multiple_of(gg * GW + j * 128, 128), 128)
        q = jnp.dot(x_v[br], wq_v[br, :, c], preferred_element_type=f32)
        q = (q * QSCALE).astype(bf16)
        h, half = j // 2, j % 2
        for b in range(B):
            q_s[br, gg, b, h * SQ:(h + 1) * SQ, half * 128:(half + 1) * 128] = q[b * SQ:(b + 1) * SQ]

    @pl.when(g == 0)
    def _():
        wq_copy(0, 0).start(priority=PLO); x_copy(0).start(priority=PLO)
        fence()
        wq_copy(1, 0).start(priority=PLO); x_copy(1).start(priority=PLO)
        fence()
        for gg in range(1, QA):
            for br in range(2):
                wq_copy(br, gg).start(priority=PLO)
        def issue(gg, lo, hi):
            if lo == 0:
                for br in range(2):
                    wo_copy(br, gg).start(priority=PLO)
                    if not (WQB4 and br == 1):
                        wq_copy(br, gg + QA).start(priority=PLO)
            elif WQB4:
                wq_copy(1, gg + QA).start(priority=PLO)
            for b in range(lo, hi):
                if gg * B + b < LA:
                    kva_start(gg, b, PLO)
                kvb_start(gg, b)

        fence()
        issue(0, 0, 4)
        fence()
        issue(0, 4, 8)
        acc[...] = jnp.zeros(acc.shape, f32)

        def qbody(i, c):
            br = i % 2
            gg = i // 2

            @pl.when(i < 2)
            def _():
                pltpu.make_async_copy(x_v.at[br], x_v.at[br], x_sem.at[br]).wait()
            wq_wait(br, gg)

            @pl.when(i == 2)
            def _():
                issue(1, 0, 4)

            @pl.when(i == 4)
            def _():
                issue(1, 4, 8)
            for j in range(4):
                qpiece(br, gg, j)
            return c
        with jax.named_scope('qloop'):
            lax.fori_loop(0, 2 * QA, qbody, 0)

    def group(main):
        waits = MWAITS if main else TWAITS
        slot = g % NSLOT
        kv = kv_v.at[slot]
        gcol = cols(g)
        gn = g + NSLOT

        @pl.when(gn < G)
        def _():
            for br in range(2):
                wo_copy(br, gn).start(priority=PLO)

        if main:
            @pl.when(gn + QA < G)
            def _():
                for br in range(1 if WQB4 else 2):
                    wq_copy(br, gn + QA).start(priority=PLO)

        def oproj(br, j):
            t = lax.dot_general(wo_v[br, :, gcol], o_s[br, j * 128:(j + 1) * 128, :], NT, preferred_element_type=f32)
            acc[br * D:(br + 1) * D, j * 128:(j + 1) * 128] += t

        def finish(j):
            if main:
                return
            out_v[j * 128:(j + 1) * 128, :] = acc[:, j * 128:(j + 1) * 128].T.astype(bf16)

        def refill(b):
            @pl.when(gn < GF)
            def _():
                kvb_start(gn, b)
            if main and WQB4 and b == 3:
                @pl.when(gn + QA < G)
                def _():
                    wq_copy(1, gn + QA).start(priority=PLO)

        def refill_a(b):
            la = LA if main else LT
            gt = g + (b + la) // B
            cond = gt < GF
            if not main:
                cond = jnp.logical_and(cond, g * B + b + la >= (G - QA) * B + LA)

            @pl.when(cond)
            def _():
                kva_start(gt, (b + la) % B, 0)

            if not main:
                @pl.when(jnp.logical_and(g + 1 >= GF, g + 1 < G))
                def _():
                    kva_start(g + 1, b, PLO)
                    kvb_start(g + 1, b)

        def do_waits(b):
            if b in waits:
                with jax.named_scope('w%d' % b):
                    nxt = min([w for w in waits if w > b] + [B])
                    for bb in range(b, nxt):
                        kv_wait(g, bb)
                    if b == 0:
                        for br in range(2):
                            wo_copy(br, g).wait()
                            if main and not (WQB4 and br == 1):
                                wq_wait(br, g + QA)
                    if b == 4 and main and WQB4:
                        wq_wait(1, g + QA)

        def oproj_half(br, j, h):
            c = pl.ds(pl.multiple_of(g * GW + h * DH, DH), DH)
            t = lax.dot_general(wo_v[br, :, c], o_s[br, j * 128:(j + 1) * 128, h * DH:(h + 1) * DH], NT, preferred_element_type=f32)
            acc[br * D:(br + 1) * D, j * 128:(j + 1) * 128] += t

        S = {}
        P = {}

        def qk(c, b):
            if c == 'a':
                S[c, b] = _qk(q_s[0, g, b], kv[b, 0])
            elif c == 'b0':
                S[c, b] = _qk(q_s[1, g, b, :SQ], kv[b, 2])
            else:
                S[c, b] = _qk(q_s[1, g, b, SQ:], kv[b, 3])

        def sm(c, b):
            P[c, b] = _softmax(S.pop((c, b)))

        def pv(c, b):
            if b < 0:
                return
            if (c, b) not in P:
                sm(c, b)
            p, l = P.pop((c, b))
            rows = slice(b * SQ, (b + 1) * SQ)
            if c == 'a':
                oa = _pv(p, l, kv[b, 1])
                o_s[0, rows, :DH] = oa[:SQ]
                o_s[0, rows, DH:] = oa[SQ:]
            elif c == 'b0':
                o_s[1, rows, :DH] = _pv(p, l, kv[b, 4])
            else:
                o_s[1, rows, DH:] = _pv(p, l, kv[b, 5])

        def op(br, j):
            if j >= 0:
                oproj(br, j)

        def out_start(js):
            @pl.when(g == G - 1)
            def _():
                for j in js:
                    out_copy(j).start()

        def attn(b, with_pend=True):
            if ORDER == 0:
                qk('a', b)
                if with_pend:
                    pv('b1', b - 1)
                qk('b0', b); pv('a', b); qk('b1', b); pv('b0', b)
            elif ORDER == 1:
                if with_pend:
                    pv('b1', b - 1)
                qk('a', b); qk('b0', b); pv('a', b); qk('b1', b); pv('b0', b)
            elif ORDER == 2:
                if with_pend:
                    pv('b1', b - 1)
                qk('a', b); qk('b0', b); qk('b1', b); pv('a', b); pv('b0', b)
            sm('b1', b)
            refill_a(b)

        if not main:
            for b in range(B):
                do_waits(b)
                if b == B - 1:
                    out_start(range(B - 2 if F5 else B - 3))
                    fence()
                    if not F5:
                        finish(B - 3)
                        out_start([B - 3])
                elif b >= 3:
                    finish(b - 3)
                attn(b, with_pend=(b < B - 1))
                if b < B - 2:
                    op(0, b - 1)
                    op(1, b - 2)
                    if b >= 1:
                        refill(b - 1)
                elif b == B - 2:
                    op(1, b - 2)
                    finish(b - 2)
                    pv('b1', b)
                    op(0, b - 1)
                    op(1, b - 1)
                    if F5:
                        finish(b - 1)
                    refill(b - 1)
                    refill(b)
                else:
                    if SPLIT:
                        oproj_half(1, b - 1, 0)
                        pv('b1', b)
                        op(0, b - 1)
                        oproj_half(1, b - 1, 1)
                    else:
                        op(0, b - 1)
                        pv('b1', b)
                        op(1, b - 1)
                    refill(b)
            finish(B - 2)
            out_start([B - 2])
            return

        for b in range(B):
            do_waits(b)
            if QFIRST and b in waits:
                qpiece(b // 4, g + QA, b % 4)
            attn(b)
            if b < B - 1 and not (QFIRST and b in waits):
                qpiece(b // 4, g + QA, b % 4)
            op(0, b - 1 if OA1 else b - 2)
            op(1, b - 2)
            if b >= 1:
                refill(b - 1)
        if not OA1:
            op(0, B - 2)
        pv('b1', B - 1)
        qpiece(1, g + QA, 3)
        op(1, B - 2)
        refill(B - 1)

    @pl.when(g < G - QA)
    def _():
        with jax.named_scope('main'):
            group(True)

    @pl.when(g >= G - QA)
    def _():
        with jax.named_scope('tail'):
            group(False)

    @pl.when(g == G - 1)
    def _():
        with jax.named_scope('outwait'):
            for j in range(7):
                out_copy(j).wait()


@jax.jit
def pallas_concat_heads__gqa_block_cached__mha_block_cached__near_ridge_kernel(A_x, A_k_cache, A_v_cache, A_wq, A_wo, B_x, B_k_cache, B_v_cache, B_wq, B_wo):
    xa = A_x.reshape(M, D)
    xb = B_x.reshape(M, D)
    hbm = pl.BlockSpec(memory_space=pltpu.MemorySpace.HBM)
    out = pl.pallas_call(
        kernel,
        grid=(G,),
        in_specs=[hbm] * 10,
        out_specs=hbm,
        out_shape=jax.ShapeDtypeStruct((M, 2 * D), bf16),
        scratch_shapes=[
            pltpu.VMEM((2, M, D), bf16),
            pltpu.VMEM((2, D, H * DH), bf16),
            pltpu.VMEM((2, D, H * DH), bf16),
            pltpu.VMEM((NSLOT, B, 6, SK, DH), bf16),
            pltpu.VMEM((2, G, B, 2 * SQ, DH), bf16),
            pltpu.VMEM((2, M, GW), bf16),
            pltpu.VMEM((2 * D, M), f32),
            pltpu.VMEM((M, 2 * D), bf16),
            pltpu.SemaphoreType.DMA((2,)),
            pltpu.SemaphoreType.DMA((2, G)),
            pltpu.SemaphoreType.DMA((2, G)),
            pltpu.SemaphoreType.DMA((NSLOT, B)),
            pltpu.SemaphoreType.DMA((7,)),
            pltpu.SemaphoreType.REGULAR,
        ],
        compiler_params=pltpu.CompilerParams(
            dimension_semantics=("arbitrary",),
            vmem_limit_bytes=100 * 1024 * 1024,
            disable_bounds_checks=True,
            disable_semaphore_checks=True,
        ),
    )(xa, A_k_cache, A_v_cache, A_wq, A_wo.T, xb, B_k_cache, B_v_cache, B_wq, B_wo.T)
    return out.reshape(B, SQ, 2 * D)
```

```python
import math

import jax
import jax.numpy as jnp
from jax import lax
import jax.experimental.pallas as pl
import jax.experimental.pallas.tpu as pltpu

B, SQ, D = 8, 112, 448
H, SK, DH = 16, 512, 256
M = B * SQ
G = 8
GW = 2 * DH
NTILE = M // 128
QSCALE = DH ** -0.5 * math.log2(math.e)
NT = (((1,), (1,)), ((), ()))
bf16 = jnp.bfloat16
f32 = jnp.float32

QA = 3
MAIN_WAITS = (0, 4)
TAIL_WAITS = (0, 2, 3, 4, 5, 6, 7)
LA_MAIN = 5
LA_TAIL = 2
HI, LO = 0, 1


def _qk(q, k):
    return lax.dot_general(q, k, NT, preferred_element_type=f32)


def _softmax(s):
    m = jnp.max(s, axis=-1, keepdims=True)
    p = jnp.exp2(s - m)
    l = jnp.sum(p, axis=-1, keepdims=True)
    return p.astype(bf16), l


def _pv(p, l, v):
    o = jnp.dot(p, v, preferred_element_type=f32)
    r = pl.reciprocal(l, approx=True)
    r = r * (2.0 - l * r)
    return (o * r).astype(bf16)


def _kernel(xa_h, ka_h, va_h, wqa_h, woa_h, xb_h, kb_h, vb_h, wqb_h, wob_h, out_h,
            x_v, wq_v, wo_v, kv_v, q_s, o_s, acc, out_v,
            x_sem, wq_sem, wo_sem, kv_sem, out_sem, fence_sem):
    g = pl.program_id(0)

    def cols(gg):
        return pl.ds(pl.multiple_of(gg * GW, GW), GW)

    def x_start(br):
        pltpu.make_async_copy((xa_h, xb_h)[br], x_v.at[br], x_sem.at[br]).start(priority=LO)

    def x_wait(br):
        pltpu.make_async_copy(x_v.at[br], x_v.at[br], x_sem.at[br]).wait()

    def wq_start(br, gg):
        pltpu.make_async_copy((wqa_h, wqb_h)[br].at[:, cols(gg)], wq_v.at[br, :, cols(gg)],
                              wq_sem.at[br, gg]).start(priority=LO)

    def wq_wait(br, gg):
        dst = wq_v.at[br, :, cols(gg)]
        pltpu.make_async_copy(dst, dst, wq_sem.at[br, gg]).wait()

    def wo_copy(br, gg):
        return pltpu.make_async_copy((woa_h, wob_h)[br].at[:, cols(gg)], wo_v.at[br, :, cols(gg)],
                                     wo_sem.at[br, gg])

    def kva_start(gg, b, priority):
        dst, sem = kv_v.at[gg % 2, b], kv_sem.at[gg % 2, b]
        pltpu.make_async_copy(ka_h.at[b, gg], dst.at[0], sem).start(priority=priority)
        pltpu.make_async_copy(va_h.at[b, gg], dst.at[1], sem).start(priority=priority)

    def kvb_start(gg, b):
        dst, sem = kv_v.at[gg % 2, b], kv_sem.at[gg % 2, b]
        heads = pl.ds(2 * gg, 2)
        pltpu.make_async_copy(kb_h.at[b, heads], dst.at[pl.ds(2, 2)], sem).start(priority=LO)
        pltpu.make_async_copy(vb_h.at[b, heads], dst.at[pl.ds(4, 2)], sem).start(priority=LO)

    def kv_wait(gg, b):
        dst = kv_v.at[gg % 2, b]
        pltpu.make_async_copy(dst, dst, kv_sem.at[gg % 2, b]).wait()

    def out_copy(j):
        rows = pl.ds(j * 128, 128)
        return pltpu.make_async_copy(out_v.at[rows], out_h.at[rows], out_sem.at[j])

    def fence():
        pl.semaphore_signal(fence_sem, 1)
        pl.semaphore_wait(fence_sem, 1)

    def qpiece(br, gg, j):
        c = pl.ds(pl.multiple_of(gg * GW + j * 128, 128), 128)
        q = jnp.dot(x_v[br], wq_v[br, :, c], preferred_element_type=f32)
        q = (q * QSCALE).astype(bf16)
        h, half = j // 2, j % 2
        for b in range(B):
            q_s[br, gg, b, h * SQ:(h + 1) * SQ, half * 128:(half + 1) * 128] = q[b * SQ:(b + 1) * SQ]

    @pl.when(g == 0)
    def _():
        def issue(gg, lo, hi):
            if lo == 0:
                wo_copy(0, gg).start(priority=LO)
                wq_start(0, gg + QA)
                wo_copy(1, gg).start(priority=LO)
            else:
                wq_start(1, gg + QA)
            for b in range(lo, hi):
                if gg * B + b < LA_MAIN:
                    kva_start(gg, b, LO)
                kvb_start(gg, b)

        for br in range(2):
            wq_start(br, 0)
            x_start(br)
            fence()
        for gg in range(1, QA):
            for br in range(2):
                wq_start(br, gg)
        fence()
        issue(0, 0, 4)
        fence()
        issue(0, 4, B)
        acc[...] = jnp.zeros(acc.shape, f32)

        def qbody(i, carry):
            br, gg = i % 2, i // 2

            @pl.when(i < 2)
            def _():
                x_wait(br)

            wq_wait(br, gg)

            @pl.when(i == 2)
            def _():
                issue(1, 0, 4)

            @pl.when(i == 4)
            def _():
                issue(1, 4, B)

            for j in range(4):
                qpiece(br, gg, j)
            return carry

        lax.fori_loop(0, 2 * QA, qbody, 0)

    def group(main):
        waits = MAIN_WAITS if main else TAIL_WAITS
        kv = kv_v.at[g % 2]
        gn = g + 2

        @pl.when(gn < G)
        def _():
            for br in range(2):
                wo_copy(br, gn).start(priority=LO)

        if main:
            @pl.when(gn + QA < G)
            def _():
                wq_start(0, gn + QA)

        def wait_data(b):
            if b not in waits:
                return
            for bb in range(b, min([w for w in waits if w > b] + [B])):
                kv_wait(g, bb)
            if b == 0:
                wo_copy(0, g).wait()
                if main:
                    wq_wait(0, g + QA)
                wo_copy(1, g).wait()
            if main and b == 4:
                wq_wait(1, g + QA)

        def refill_b(b):
            @pl.when(gn < G - 1)
            def _():
                kvb_start(gn, b)

            if main and b == 3:
                @pl.when(gn + QA < G)
                def _():
                    wq_start(1, gn + QA)

        def refill_a(b):
            la = LA_MAIN if main else LA_TAIL
            gt = g + (b + la) // B
            cond = gt < G - 1
            if not main:
                cond = jnp.logical_and(cond, g * B + b + la >= (G - QA) * B + LA_MAIN)

            @pl.when(cond)
            def _():
                kva_start(gt, (b + la) % B, HI)

            if not main:
                @pl.when(g == G - 2)
                def _():
                    kva_start(G - 1, b, LO)
                    kvb_start(G - 1, b)

        scores, probs = {}, {}

        def qk(c, b):
            if c == 'a':
                scores[c, b] = _qk(q_s[0, g, b], kv[b, 0])
            elif c == 'b0':
                scores[c, b] = _qk(q_s[1, g, b, :SQ], kv[b, 2])
            else:
                scores[c, b] = _qk(q_s[1, g, b, SQ:], kv[b, 3])

        def softmax(c, b):
            probs[c, b] = _softmax(scores.pop((c, b)))

        def pv(c, b):
            if (c, b) not in probs:
                softmax(c, b)
            p, l = probs.pop((c, b))
            rows = slice(b * SQ, (b + 1) * SQ)
            if c == 'a':
                oa = _pv(p, l, kv[b, 1])
                o_s[0, rows, :DH] = oa[:SQ]
                o_s[0, rows, DH:] = oa[SQ:]
            elif c == 'b0':
                o_s[1, rows, :DH] = _pv(p, l, kv[b, 4])
            else:
                o_s[1, rows, DH:] = _pv(p, l, kv[b, 5])

        def attention(b, pending):
            if pending:
                pv('b1', b - 1)
            qk('a', b)
            qk('b0', b)
            pv('a', b)
            qk('b1', b)
            pv('b0', b)
            softmax('b1', b)
            refill_a(b)

        def oproj(br, j):
            if j < 0:
                return
            toks = slice(j * 128, (j + 1) * 128)
            t = lax.dot_general(wo_v[br, :, cols(g)], o_s[br, toks, :], NT, preferred_element_type=f32)
            acc[br * D:(br + 1) * D, toks] += t

        def finish(j):
            toks = slice(j * 128, (j + 1) * 128)
            out_v[toks, :] = acc[:, toks].T.astype(bf16)

        def out_start(tiles):
            @pl.when(g == G - 1)
            def _():
                for j in tiles:
                    out_copy(j).start()

        if main:
            for b in range(B):
                wait_data(b)
                if b in waits:
                    qpiece(b // 4, g + QA, b % 4)
                attention(b, pending=b > 0)
                if b not in waits and b < B - 1:
                    qpiece(b // 4, g + QA, b % 4)
                oproj(0, b - 1)
                oproj(1, b - 2)
                if b >= 1:
                    refill_b(b - 1)
            pv('b1', B - 1)
            qpiece(1, g + QA, 3)
            oproj(1, B - 2)
            refill_b(B - 1)
            return

        for b in range(B - 2):
            wait_data(b)
            if b >= 3:
                finish(b - 3)
            attention(b, pending=b > 0)
            oproj(0, b - 1)
            oproj(1, b - 2)
            if b >= 1:
                refill_b(b - 1)
        b = B - 2
        wait_data(b)
        finish(b - 3)
        attention(b, pending=True)
        oproj(1, b - 2)
        finish(b - 2)
        pv('b1', b)
        oproj(0, b - 1)
        oproj(1, b - 1)
        refill_b(b - 1)
        refill_b(b)
        b = B - 1
        wait_data(b)
        out_start(range(NTILE - 2))
        fence()
        finish(NTILE - 2)
        out_start([NTILE - 2])
        attention(b, pending=False)
        oproj(0, b - 1)
        pv('b1', b)
        oproj(1, b - 1)
        refill_b(b)
        finish(NTILE - 1)
        out_start([NTILE - 1])

    @pl.when(g < G - QA)
    def _():
        group(main=True)

    @pl.when(g >= G - QA)
    def _():
        group(main=False)

    @pl.when(g == G - 1)
    def _():
        for j in range(NTILE):
            out_copy(j).wait()


@jax.jit
def pallas_concat_heads__gqa_block_cached__mha_block_cached__near_ridge_kernel(
    A_x: jax.Array,
    A_k_cache: jax.Array,
    A_v_cache: jax.Array,
    A_wq: jax.Array,
    A_wo: jax.Array,
    B_x: jax.Array,
    B_k_cache: jax.Array,
    B_v_cache: jax.Array,
    B_wq: jax.Array,
    B_wo: jax.Array,
):
    hbm = pl.BlockSpec(memory_space=pltpu.MemorySpace.HBM)
    out = pl.pallas_call(
        _kernel,
        grid=(G,),
        in_specs=[hbm] * 10,
        out_specs=hbm,
        out_shape=jax.ShapeDtypeStruct((M, 2 * D), bf16),
        scratch_shapes=[
            pltpu.VMEM((2, M, D), bf16),
            pltpu.VMEM((2, D, H * DH), bf16),
            pltpu.VMEM((2, D, H * DH), bf16),
            pltpu.VMEM((2, B, 6, SK, DH), bf16),
            pltpu.VMEM((2, G, B, 2 * SQ, DH), bf16),
            pltpu.VMEM((2, M, GW), bf16),
            pltpu.VMEM((2 * D, M), f32),
            pltpu.VMEM((M, 2 * D), bf16),
            pltpu.SemaphoreType.DMA((2,)),
            pltpu.SemaphoreType.DMA((2, G)),
            pltpu.SemaphoreType.DMA((2, G)),
            pltpu.SemaphoreType.DMA((2, B)),
            pltpu.SemaphoreType.DMA((NTILE,)),
            pltpu.SemaphoreType.REGULAR,
        ],
        compiler_params=pltpu.CompilerParams(
            dimension_semantics=("arbitrary",),
            vmem_limit_bytes=100 * 1024 * 1024,
            disable_bounds_checks=True,
            disable_semaphore_checks=True,
        ),
    )(A_x.reshape(M, D), A_k_cache, A_v_cache, A_wq, A_wo.T,
      B_x.reshape(M, D), B_k_cache, B_v_cache, B_wq, B_wo.T)
    return out.reshape(B, SQ, 2 * D)
```

```python
import math

import jax
import jax.numpy as jnp
from jax import lax
import jax.experimental.pallas as pl
import jax.experimental.pallas.tpu as pltpu

B, SQ, D = 8, 112, 448
H, SK, DH = 16, 512, 256
M = B * SQ
G = 8
GW = 2 * DH
NTILE = M // 128
QSCALE = DH ** -0.5 * math.log2(math.e)
NT = (((1,), (1,)), ((), ()))
bf16 = jnp.bfloat16
f32 = jnp.float32

QA = 3
MAIN_WAITS = (0, 4)
TAIL_WAITS = tuple(range(B))
MAIN_A_SCHEDULE = {0: (4, 5), 1: (6,), 2: (7,), 4: (8, 9), 5: (10,), 6: (11,)}
LA_TAIL = 2
HI, LO = 0, 1


def _qk(q, k):
    return lax.dot_general(q, k, NT, preferred_element_type=f32)


def _softmax(s):
    m = jnp.max(s, axis=-1, keepdims=True)
    p = jnp.exp2(s - m)
    l = jnp.sum(p, axis=-1, keepdims=True)
    return p.astype(bf16), l


def _pv(p, l, v):
    o = jnp.dot(p, v, preferred_element_type=f32)
    r = pl.reciprocal(l, approx=True)
    r = r * (2.0 - l * r)
    return (o * r).astype(bf16)


def _kernel(xa_h, ka_h, va_h, wqa_h, woa_h, xb_h, kb_h, vb_h, wqb_h, wob_h, out_h,
            x_v, wq_v, wo_v, kv_v, q_s, o_s, acc, out_v,
            x_sem, wq_sem, wo_sem, kv_sem, out_sem, fence_sem):
    g = pl.program_id(0)

    def cols(gg):
        return pl.ds(pl.multiple_of(gg * GW, GW), GW)

    def x_copy(br, part):
        rows = pl.ds(part * (M // 2), M // 2)
        return pltpu.make_async_copy((xa_h, xb_h)[br].at[rows], x_v.at[br, rows], x_sem.at[br, part])

    def wq_start(br, gg):
        pltpu.make_async_copy((wqa_h, wqb_h)[br].at[:, cols(gg)], wq_v.at[br, :, cols(gg)],
                              wq_sem.at[br, gg]).start(priority=LO)

    def wq_wait(br, gg):
        dst = wq_v.at[br, :, cols(gg)]
        pltpu.make_async_copy(dst, dst, wq_sem.at[br, gg]).wait()

    def wo_copy(br, gg):
        return pltpu.make_async_copy((woa_h, wob_h)[br].at[:, cols(gg)], wo_v.at[br, :, cols(gg)],
                                     wo_sem.at[br, gg])

    def kva_start(gg, b, priority):
        dst, sem = kv_v.at[gg % 2, b], kv_sem.at[gg % 2, b]
        pltpu.make_async_copy(ka_h.at[b, gg], dst.at[0], sem).start(priority=priority)
        pltpu.make_async_copy(va_h.at[b, gg], dst.at[1], sem).start(priority=priority)

    def kvb_start(gg, b):
        dst, sem = kv_v.at[gg % 2, b], kv_sem.at[gg % 2, b]
        heads = pl.ds(2 * gg, 2)
        pltpu.make_async_copy(kb_h.at[b, heads], dst.at[pl.ds(2, 2)], sem).start(priority=LO)
        pltpu.make_async_copy(vb_h.at[b, heads], dst.at[pl.ds(4, 2)], sem).start(priority=LO)

    def kv_wait(gg, b):
        dst = kv_v.at[gg % 2, b]
        pltpu.make_async_copy(dst, dst, kv_sem.at[gg % 2, b]).wait()

    def out_copy(j):
        rows = pl.ds(j * 128, 128)
        return pltpu.make_async_copy(out_v.at[rows], out_h.at[rows], out_sem.at[j])

    def fence():
        pl.semaphore_signal(fence_sem, 1)
        pl.semaphore_wait(fence_sem, 1)

    def qpiece(br, gg, j, b0=0, b1=B):
        c = pl.ds(pl.multiple_of(gg * GW + j * 128, 128), 128)
        q = jnp.dot(x_v[br, b0 * SQ:b1 * SQ], wq_v[br, :, c], preferred_element_type=f32)
        q = (q * QSCALE).astype(bf16)
        h, half = j // 2, j % 2
        for b in range(b0, b1):
            q_s[br, gg, b, h * SQ:(h + 1) * SQ, half * 128:(half + 1) * 128] = q[(b - b0) * SQ:(b - b0 + 1) * SQ]

    @pl.when(g == 0)
    def _():
        def issue(gg, lo, hi):
            if lo == 0:
                wo_copy(0, gg).start(priority=LO)
                wq_start(0, gg + QA)
                wo_copy(1, gg).start(priority=LO)
            else:
                wq_start(1, gg + QA)
            for b in range(lo, hi):
                if gg * B + b < B // 2:
                    kva_start(gg, b, LO)
                kvb_start(gg, b)

        wq_start(0, 0)
        x_copy(0, 0).start(priority=LO)
        fence()
        x_copy(0, 1).start(priority=LO)
        fence()
        wq_start(1, 0)
        x_copy(1, 0).start(priority=LO)
        x_copy(1, 1).start(priority=LO)
        fence()
        for gg in range(1, QA):
            for br in range(2):
                wq_start(br, gg)
        fence()
        issue(0, 0, 4)
        fence()
        issue(0, 4, B)
        acc[...] = jnp.zeros(acc.shape, f32)

        wq_wait(0, 0)
        for part in range(2):
            x_copy(0, part).wait()
            for j in range(4):
                qpiece(0, 0, j, part * B // 2, (part + 1) * B // 2)

        def qbody(i, carry):
            br, gg = i % 2, i // 2

            @pl.when(i == 1)
            def _():
                x_copy(1, 0).wait()
                x_copy(1, 1).wait()

            wq_wait(br, gg)

            @pl.when(i == 2)
            def _():
                issue(1, 0, 4)

            @pl.when(i == 4)
            def _():
                issue(1, 4, B)

            for j in range(4):
                qpiece(br, gg, j)
            return carry

        lax.fori_loop(1, 2 * QA, qbody, 0)

    def group(main):
        waits = MAIN_WAITS if main else TAIL_WAITS
        kv = kv_v.at[g % 2]
        gn = g + 2

        @pl.when(gn < G)
        def _():
            for br in range(2):
                wo_copy(br, gn).start(priority=LO)

        if main:
            @pl.when(gn + QA < G)
            def _():
                wq_start(0, gn + QA)

        def wait_data(b):
            if b not in waits:
                return
            for bb in range(b, min([w for w in waits if w > b] + [B])):
                kv_wait(g, bb)
            if b == 0:
                wo_copy(0, g).wait()
                if main:
                    wq_wait(0, g + QA)
                wo_copy(1, g).wait()
            if main and b == 4:
                wq_wait(1, g + QA)

        def refill_b(b):
            @pl.when(gn < G - 1)
            def _():
                kvb_start(gn, b)

            if main and b == 3:
                @pl.when(gn + QA < G)
                def _():
                    wq_start(1, gn + QA)

        def refill_a(b):
            if main:
                for c in MAIN_A_SCHEDULE.get(b, ()):
                    kva_start(g + c // B, c % B, HI)
                return
            gt = g + (b + LA_TAIL) // B
            cond = jnp.logical_and(gt < G - 1, g * B + b + LA_TAIL >= (G - QA) * B + B // 2)

            @pl.when(cond)
            def _():
                kva_start(gt, (b + LA_TAIL) % B, HI)

            @pl.when(g == G - 2)
            def _():
                kva_start(G - 1, b, LO)
                kvb_start(G - 1, b)

        scores, probs = {}, {}

        def qk(c, b):
            if c == 'a':
                scores[c, b] = _qk(q_s[0, g, b], kv[b, 0])
            elif c == 'b0':
                scores[c, b] = _qk(q_s[1, g, b, :SQ], kv[b, 2])
            else:
                scores[c, b] = _qk(q_s[1, g, b, SQ:], kv[b, 3])

        def softmax(c, b):
            probs[c, b] = _softmax(scores.pop((c, b)))

        def pv(c, b):
            if (c, b) not in probs:
                softmax(c, b)
            p, l = probs.pop((c, b))
            rows = slice(b * SQ, (b + 1) * SQ)
            if c == 'a':
                oa = _pv(p, l, kv[b, 1])
                o_s[0, rows, :DH] = oa[:SQ]
                o_s[0, rows, DH:] = oa[SQ:]
            elif c == 'b0':
                o_s[1, rows, :DH] = _pv(p, l, kv[b, 4])
            else:
                o_s[1, rows, DH:] = _pv(p, l, kv[b, 5])

        def attention(b, pending):
            if pending:
                pv('b1', b - 1)
            qk('a', b)
            qk('b0', b)
            pv('a', b)
            qk('b1', b)
            pv('b0', b)
            softmax('b1', b)
            refill_a(b)

        def oproj(br, j):
            if j < 0:
                return
            toks = slice(j * 128, (j + 1) * 128)
            t = lax.dot_general(wo_v[br, :, cols(g)], o_s[br, toks, :], NT, preferred_element_type=f32)
            acc[br * D:(br + 1) * D, toks] += t

        def finish(j):
            toks = slice(j * 128, (j + 1) * 128)
            out_v[toks, :] = acc[:, toks].T.astype(bf16)

        def out_start(tiles):
            @pl.when(g == G - 1)
            def _():
                for j in tiles:
                    out_copy(j).start()

        if main:
            for b in range(B):
                wait_data(b)
                if b in waits:
                    qpiece(b // 4, g + QA, b % 4)
                attention(b, pending=b > 0)
                if b not in waits and b < B - 1:
                    qpiece(b // 4, g + QA, b % 4)
                oproj(0, b - 1)
                oproj(1, b - 2)
                if b >= 1:
                    refill_b(b - 1)
            pv('b1', B - 1)
            qpiece(1, g + QA, 3)
            oproj(1, B - 2)
            refill_b(B - 1)
            return

        for b in range(B):
            wait_data(b)
            if b == B - 1:
                out_start(range(NTILE - 2))
                fence()
            if b >= 2:
                finish(b - 2)
            if b == B - 1:
                out_start([NTILE - 2])
            for c in ('a', 'b0', 'b1'):
                qk(c, b)
            for c in ('a', 'b0', 'b1'):
                pv(c, b)
            refill_a(b)
            oproj(0, b - 1)
            oproj(1, b - 1)
            refill_b(b)
        finish(NTILE - 1)
        out_start([NTILE - 1])

    @pl.when(g < G - QA)
    def _():
        group(main=True)

    @pl.when(g >= G - QA)
    def _():
        group(main=False)

    @pl.when(g == G - 1)
    def _():
        for j in range(NTILE):
            out_copy(j).wait()


@jax.jit
def pallas_concat_heads__gqa_block_cached__mha_block_cached__near_ridge_kernel(
    A_x: jax.Array,
    A_k_cache: jax.Array,
    A_v_cache: jax.Array,
    A_wq: jax.Array,
    A_wo: jax.Array,
    B_x: jax.Array,
    B_k_cache: jax.Array,
    B_v_cache: jax.Array,
    B_wq: jax.Array,
    B_wo: jax.Array,
):
    hbm = pl.BlockSpec(memory_space=pltpu.MemorySpace.HBM)
    out = pl.pallas_call(
        _kernel,
        grid=(G,),
        in_specs=[hbm] * 10,
        out_specs=hbm,
        out_shape=jax.ShapeDtypeStruct((M, 2 * D), bf16),
        scratch_shapes=[
            pltpu.VMEM((2, M, D), bf16),
            pltpu.VMEM((2, D, H * DH), bf16),
            pltpu.VMEM((2, D, H * DH), bf16),
            pltpu.VMEM((2, B, 6, SK, DH), bf16),
            pltpu.VMEM((2, G, B, 2 * SQ, DH), bf16),
            pltpu.VMEM((2, M, GW), bf16),
            pltpu.VMEM((2 * D, M), f32),
            pltpu.VMEM((M, 2 * D), bf16),
            pltpu.SemaphoreType.DMA((2, 2)),
            pltpu.SemaphoreType.DMA((2, G)),
            pltpu.SemaphoreType.DMA((2, G)),
            pltpu.SemaphoreType.DMA((2, B)),
            pltpu.SemaphoreType.DMA((NTILE,)),
            pltpu.SemaphoreType.REGULAR,
        ],
        compiler_params=pltpu.CompilerParams(
            dimension_semantics=("arbitrary",),
            vmem_limit_bytes=100 * 1024 * 1024,
            disable_bounds_checks=True,
            disable_semaphore_checks=True,
        ),
    )(A_x.reshape(M, D), A_k_cache, A_v_cache, A_wq, A_wo.T,
      B_x.reshape(M, D), B_k_cache, B_v_cache, B_wq, B_wo.T)
    return out.reshape(B, SQ, 2 * D)
```

```python
import jax
import jax.numpy as jnp
from jax import lax
import jax.experimental.pallas as pl
import jax.experimental.pallas.tpu as pltpu

B, SQ, D = 8, 112, 448
H, SK, DH = 16, 512, 256
M = B * SQ
G = 8
GW = 2 * DH
NTILE = M // 128
QSCALE = DH ** -0.5
NT = (((1,), (1,)), ((), ()))
bf16 = jnp.bfloat16
f32 = jnp.float32

QA = 3
MAIN_WAITS = (0, 4)
TAIL_WAITS = tuple(range(B))
MAIN_A_SCHEDULE = {0: (4, 5), 1: (6,), 2: (7,), 4: (8, 9), 5: (10,), 6: (11,)}
LA_TAIL = 1
HI, LO = 0, 1


def _qk(q, k):
    return lax.dot_general(q, k, NT, preferred_element_type=f32)


def _softmax(s):
    m = jnp.max(s, axis=-1, keepdims=True)
    p = jnp.exp(s - m)
    l = jnp.sum(p, axis=-1, keepdims=True)
    return p.astype(bf16), l


def _pv(p, l, v):
    o = jnp.dot(p, v, preferred_element_type=f32)
    r = pl.reciprocal(l, approx=True)
    r = r * (2.0 - l * r)
    return (o * r).astype(bf16)


def _kernel(xa_h, ka_h, va_h, wqa_h, woa_h, xb_h, kb_h, vb_h, wqb_h, wob_h, out_h,
            x_v, wq_v, wo_v, kv_v, q_s, o_s, acc, out_v,
            x_sem, wq_sem, wo_sem, kv_sem, out_sem, fence_sem):
    g = pl.program_id(0)

    def cols(gg):
        return pl.ds(pl.multiple_of(gg * GW, GW), GW)

    def x_copy(br, part):
        rows = pl.ds(part * (M // 2), M // 2)
        return pltpu.make_async_copy((xa_h, xb_h)[br].at[rows], x_v.at[br, rows], x_sem.at[br, part])

    def wq_start(br, gg):
        pltpu.make_async_copy((wqa_h, wqb_h)[br].at[:, cols(gg)], wq_v.at[br, :, cols(gg)],
                              wq_sem.at[br, gg]).start(priority=LO)

    def wq_wait(br, gg):
        dst = wq_v.at[br, :, cols(gg)]
        pltpu.make_async_copy(dst, dst, wq_sem.at[br, gg]).wait()

    def wo_copy(br, gg):
        return pltpu.make_async_copy((woa_h, wob_h)[br].at[:, cols(gg)], wo_v.at[br, :, cols(gg)],
                                     wo_sem.at[br, gg])

    def kva_start(gg, b, priority):
        dst, sem = kv_v.at[gg % 2, b], kv_sem.at[gg % 2, b]
        pltpu.make_async_copy(ka_h.at[b, gg], dst.at[0], sem).start(priority=priority)
        pltpu.make_async_copy(va_h.at[b, gg], dst.at[1], sem).start(priority=priority)

    def kvb_start(gg, b):
        dst, sem = kv_v.at[gg % 2, b], kv_sem.at[gg % 2, b]
        heads = pl.ds(2 * gg, 2)
        pltpu.make_async_copy(kb_h.at[b, heads], dst.at[pl.ds(2, 2)], sem).start(priority=LO)
        pltpu.make_async_copy(vb_h.at[b, heads], dst.at[pl.ds(4, 2)], sem).start(priority=LO)

    def kv_wait(gg, b):
        dst = kv_v.at[gg % 2, b]
        pltpu.make_async_copy(dst, dst, kv_sem.at[gg % 2, b]).wait()

    def out_copy(j):
        rows = pl.ds(j * 128, 128)
        return pltpu.make_async_copy(out_v.at[rows], out_h.at[rows], out_sem.at[j])

    def fence():
        pl.semaphore_signal(fence_sem, 1)
        pl.semaphore_wait(fence_sem, 1)

    def qpiece(br, gg, j, b0=0, b1=B):
        c = pl.ds(pl.multiple_of(gg * GW + j * 128, 128), 128)
        q = jnp.dot(x_v[br, b0 * SQ:b1 * SQ], wq_v[br, :, c], preferred_element_type=f32)
        q = (q * QSCALE).astype(bf16)
        h, half = j // 2, j % 2
        for b in range(b0, b1):
            q_s[br, gg, b, h * SQ:(h + 1) * SQ, half * 128:(half + 1) * 128] = q[(b - b0) * SQ:(b - b0 + 1) * SQ]

    @pl.when(g == 0)
    def _():
        def issue(gg, lo, hi):
            if lo == 0:
                wo_copy(0, gg).start(priority=LO)
                wq_start(0, gg + QA)
                wo_copy(1, gg).start(priority=LO)
            else:
                wq_start(1, gg + QA)
            for b in range(lo, hi):
                if gg * B + b < B // 2:
                    kva_start(gg, b, LO)
                kvb_start(gg, b)

        wq_start(0, 0)
        x_copy(0, 0).start(priority=LO)
        fence()
        x_copy(0, 1).start(priority=LO)
        fence()
        wq_start(1, 0)
        x_copy(1, 0).start(priority=LO)
        x_copy(1, 1).start(priority=LO)
        fence()
        for gg in range(1, QA):
            for br in range(2):
                wq_start(br, gg)
        fence()
        issue(0, 0, 4)
        fence()
        issue(0, 4, B)
        acc[...] = jnp.zeros(acc.shape, f32)

        wq_wait(0, 0)
        for part in range(2):
            x_copy(0, part).wait()
            for j in range(4):
                qpiece(0, 0, j, part * B // 2, (part + 1) * B // 2)

        def qbody(i, carry):
            br, gg = i % 2, i // 2

            @pl.when(i == 1)
            def _():
                x_copy(1, 0).wait()
                x_copy(1, 1).wait()

            wq_wait(br, gg)

            @pl.when(i == 2)
            def _():
                issue(1, 0, 4)

            @pl.when(i == 4)
            def _():
                issue(1, 4, B)

            for j in range(4):
                qpiece(br, gg, j)
            return carry

        lax.fori_loop(1, 2 * QA, qbody, 0)

    def group(main):
        waits = MAIN_WAITS if main else TAIL_WAITS
        kv = kv_v.at[g % 2]
        gn = g + 2

        @pl.when(gn < G)
        def _():
            for br in range(2):
                wo_copy(br, gn).start(priority=LO)

        if main:
            @pl.when(gn + QA < G)
            def _():
                wq_start(0, gn + QA)

        def wait_data(b):
            if b not in waits:
                return
            for bb in range(b, min([w for w in waits if w > b] + [B])):
                kv_wait(g, bb)
            if b == 0:
                wo_copy(0, g).wait()
                if main:
                    wq_wait(0, g + QA)
                wo_copy(1, g).wait()
            if main and b == 4:
                wq_wait(1, g + QA)

        def refill_b(b):
            @pl.when(gn < G)
            def _():
                kvb_start(gn, b)

            if main and b == 3:
                @pl.when(gn + QA < G)
                def _():
                    wq_start(1, gn + QA)

        def refill_a(b):
            if main:
                for c in MAIN_A_SCHEDULE.get(b, ()):
                    kva_start(g + c // B, c % B, HI)
                return
            gt = g + (b + LA_TAIL) // B
            cond = jnp.logical_and(gt < G, g * B + b + LA_TAIL >= (G - QA) * B + B // 2)

            @pl.when(cond)
            def _():
                kva_start(gt, (b + LA_TAIL) % B, HI)

        scores, probs = {}, {}

        def qk(c, b):
            if c == 'a':
                scores[c, b] = _qk(q_s[0, g, b], kv[b, 0])
            elif c == 'b0':
                scores[c, b] = _qk(q_s[1, g, b, :SQ], kv[b, 2])
            else:
                scores[c, b] = _qk(q_s[1, g, b, SQ:], kv[b, 3])

        def softmax(c, b):
            probs[c, b] = _softmax(scores.pop((c, b)))

        def pv(c, b):
            if (c, b) not in probs:
                softmax(c, b)
            p, l = probs.pop((c, b))
            rows = slice(b * SQ, (b + 1) * SQ)
            if c == 'a':
                oa = _pv(p, l, kv[b, 1])
                o_s[0, rows, :DH] = oa[:SQ]
                o_s[0, rows, DH:] = oa[SQ:]
            elif c == 'b0':
                o_s[1, rows, :DH] = _pv(p, l, kv[b, 4])
            else:
                o_s[1, rows, DH:] = _pv(p, l, kv[b, 5])

        def attention(b, pending):
            if pending:
                pv('b1', b - 1)
            qk('a', b)
            qk('b0', b)
            pv('a', b)
            qk('b1', b)
            pv('b0', b)
            softmax('b1', b)
            refill_a(b)

        def oproj(br, j):
            if j < 0:
                return
            toks = slice(j * 128, (j + 1) * 128)
            t = lax.dot_general(wo_v[br, :, cols(g)], o_s[br, toks, :], NT, preferred_element_type=f32)
            acc[br * D:(br + 1) * D, toks] += t

        def finish(j):
            toks = slice(j * 128, (j + 1) * 128)
            out_v[toks, :] = acc[:, toks].T.astype(bf16)

        def out_start(tiles):
            @pl.when(g == G - 1)
            def _():
                for j in tiles:
                    out_copy(j).start()

        if main:
            for b in range(B):
                wait_data(b)
                if b in waits:
                    qpiece(b // 4, g + QA, b % 4)
                attention(b, pending=b > 0)
                if b not in waits and b < B - 1:
                    qpiece(b // 4, g + QA, b % 4)
                oproj(0, b - 1)
                oproj(1, b - 2)
                if b >= 1:
                    refill_b(b - 1)
            pv('b1', B - 1)
            qpiece(1, g + QA, 3)
            oproj(1, B - 2)
            refill_b(B - 1)
            return

        for b in range(B):
            wait_data(b)
            refill_a(b)
            if b == B - 1:
                out_start(range(NTILE - 2))
                fence()
            if b >= 2:
                finish(b - 2)
            if b == B - 1:
                out_start([NTILE - 2])
            for c in ('a', 'b0', 'b1'):
                qk(c, b)
            for c in ('a', 'b0', 'b1'):
                pv(c, b)
            oproj(0, b - 1)
            oproj(1, b - 1)
            refill_b(b)
        finish(NTILE - 1)
        out_start([NTILE - 1])

    @pl.when(g < G - QA)
    def _():
        group(main=True)

    @pl.when(g >= G - QA)
    def _():
        group(main=False)

    @pl.when(g == G - 1)
    def _():
        for j in range(NTILE):
            out_copy(j).wait()


@jax.jit
def pallas_concat_heads__gqa_block_cached__mha_block_cached__near_ridge_kernel(
    A_x: jax.Array,
    A_k_cache: jax.Array,
    A_v_cache: jax.Array,
    A_wq: jax.Array,
    A_wo: jax.Array,
    B_x: jax.Array,
    B_k_cache: jax.Array,
    B_v_cache: jax.Array,
    B_wq: jax.Array,
    B_wo: jax.Array,
):
    hbm = pl.BlockSpec(memory_space=pltpu.MemorySpace.HBM)
    out = pl.pallas_call(
        _kernel,
        grid=(G,),
        in_specs=[hbm] * 10,
        out_specs=hbm,
        out_shape=jax.ShapeDtypeStruct((M, 2 * D), bf16),
        scratch_shapes=[
            pltpu.VMEM((2, M, D), bf16),
            pltpu.VMEM((2, D, H * DH), bf16),
            pltpu.VMEM((2, D, H * DH), bf16),
            pltpu.VMEM((2, B, 6, SK, DH), bf16),
            pltpu.VMEM((2, G, B, 2 * SQ, DH), bf16),
            pltpu.VMEM((2, M, GW), bf16),
            pltpu.VMEM((2 * D, M), f32),
            pltpu.VMEM((M, 2 * D), bf16),
            pltpu.SemaphoreType.DMA((2, 2)),
            pltpu.SemaphoreType.DMA((2, G)),
            pltpu.SemaphoreType.DMA((2, G)),
            pltpu.SemaphoreType.DMA((2, B)),
            pltpu.SemaphoreType.DMA((NTILE,)),
            pltpu.SemaphoreType.REGULAR,
        ],
        compiler_params=pltpu.CompilerParams(
            dimension_semantics=("arbitrary",),
            vmem_limit_bytes=100 * 1024 * 1024,
            disable_bounds_checks=True,
            disable_semaphore_checks=True,
        ),
    )(A_x.reshape(M, D), A_k_cache, A_v_cache, A_wq, A_wo.T,
      B_x.reshape(M, D), B_k_cache, B_v_cache, B_wq, B_wo.T)
    return out.reshape(B, SQ, 2 * D)
```

```python
import jax
import jax.numpy as jnp
from jax import lax
import jax.experimental.pallas as pl
import jax.experimental.pallas.tpu as pltpu

B, SQ, D = 8, 112, 448
H, SK, DH = 16, 512, 256
M = B * SQ
G = 8
GW = 2 * DH
HALF = B // 2
NTILE = M // 128
QSCALE = DH ** -0.5
NT = (((1,), (1,)), ((), ()))
bf16 = jnp.bfloat16
f32 = jnp.float32

QA = 3
MAIN_WAITS = (0, 4)
TAIL_WAITS = (0, 2, 3, 4, 5, 6, 7)
MAIN_A_SCHEDULE = {0: (4, 5), 1: (6,), 2: (7,), 4: (8, 9), 5: (10,), 6: (11,)}
LA_TAIL = 1
NPM = 8
NPT = 4
PAIR = 0
EM = 4
ET = 2
MID_SPAN = 2
HI, LO = 0, 1


def _qk(q, k):
    return lax.dot_general(q, k, NT, preferred_element_type=f32)


def _softmax(s):
    m = jnp.max(s, axis=-1, keepdims=True)
    p = jnp.exp(s - m)
    l = jnp.sum(p, axis=-1, keepdims=True)
    return p.astype(bf16), l


def _pv(p, l, v):
    o = jnp.dot(p, v, preferred_element_type=f32)
    r = pl.reciprocal(l, approx=True)
    r = r * (2.0 - l * r)
    return (o * r).astype(bf16)


def _kernel(xa_h, ka_h, va_h, wqa_h, woa_h, xb_h, kb_h, vb_h, wqb_h, wob_h, out_h,
            x_v, wq_v, wo_v, kv_v, q_s, oa_s, ob_s, acc, fin_s, out_v,
            x_sem, wq_sem, wo_sem, kv_sem, out_sem, fence_sem):
    g = pl.program_id(0)

    def cols(gg):
        return pl.ds(pl.multiple_of(gg * GW, GW), GW)

    def x_copy(br, part):
        rows = pl.ds(part * (M // 2), M // 2)
        return pltpu.make_async_copy((xa_h, xb_h)[br].at[rows], x_v.at[br, rows], x_sem.at[br, part])

    def wq_start(br, gg):
        pltpu.make_async_copy((wqa_h, wqb_h)[br].at[:, cols(gg)], wq_v.at[br, :, cols(gg)],
                              wq_sem.at[br, gg]).start(priority=LO)

    def wq_wait(br, gg):
        dst = wq_v.at[br, :, cols(gg)]
        pltpu.make_async_copy(dst, dst, wq_sem.at[br, gg]).wait()

    def wo_copy(br, gg):
        return pltpu.make_async_copy((woa_h, wob_h)[br].at[:, cols(gg)], wo_v.at[br, :, cols(gg)],
                                     wo_sem.at[br, gg])

    def chunk_sem(gg, b):
        if isinstance(gg, int):
            i = b // HALF * HALF if gg < G - QA else b
        else:
            i = jnp.where(gg < G - QA, b // HALF * HALF, b)
        return kv_sem.at[gg % 2, i]

    def kva_piece(gg, b, i, NP):
        rows = pl.ds((i % NP) * (SK // NP), SK // NP)
        src = (ka_h, va_h)[i // NP]
        pltpu.make_async_copy(src.at[b, gg, rows], kv_v.at[gg % 2, b, i // NP, rows],
                              chunk_sem(gg, b)).start(priority=HI)

    def kva_start(gg, b, n):
        dst, sem, bs = kv_v.at[gg % 2, pl.ds(b, n)], chunk_sem(gg, b), pl.ds(b, n)
        pltpu.make_async_copy(ka_h.at[bs, gg], dst.at[:, 0], sem).start(priority=LO)
        pltpu.make_async_copy(va_h.at[bs, gg], dst.at[:, 1], sem).start(priority=LO)

    def kvb_start(gg, b, n=1):
        dst, sem, bs = kv_v.at[gg % 2, pl.ds(b, n)], chunk_sem(gg, b), pl.ds(b, n)
        heads = pl.ds(2 * gg, 2)
        pltpu.make_async_copy(kb_h.at[bs, heads], dst.at[:, pl.ds(2, 2)], sem).start(priority=LO)
        pltpu.make_async_copy(vb_h.at[bs, heads], dst.at[:, pl.ds(4, 2)], sem).start(priority=LO)

    def kv_wait(gg, b, n):
        dst = kv_v.at[gg % 2, pl.ds(b, n)]
        pltpu.make_async_copy(dst, dst, kv_sem.at[gg % 2, b]).wait()

    def out_copy(j):
        rows = pl.ds(j * 128, 128)
        return pltpu.make_async_copy(out_v.at[rows], out_h.at[rows], out_sem.at[j])

    def fence():
        pl.semaphore_signal(fence_sem, 1)
        pl.semaphore_wait(fence_sem, 1)

    def qpiece(br, gg, j, b0=0, b1=B):
        c = pl.ds(pl.multiple_of(gg * GW + j * 128, 128), 128)
        q = jnp.dot(x_v[br, b0 * SQ:b1 * SQ], wq_v[br, :, c], preferred_element_type=f32)
        q = (q * QSCALE).astype(bf16)
        h, half = j // 2, j % 2
        for b in range(b0, b1):
            q_s[br, gg, b, h * SQ:(h + 1) * SQ, half * 128:(half + 1) * 128] = q[(b - b0) * SQ:(b - b0 + 1) * SQ]

    @pl.when(g == 0)
    def _():
        def issue(gg, lo, hi):
            if lo == 0:
                wo_copy(0, gg).start(priority=LO)
                wq_start(0, gg + QA)
                wo_copy(1, gg).start(priority=LO)
            else:
                wq_start(1, gg + QA)
            if gg == 0 and lo == 0:
                kva_start(gg, lo, HALF)
            kvb_start(gg, lo, HALF)

        wq_start(0, 0)
        x_copy(0, 0).start(priority=LO)
        fence()
        x_copy(0, 1).start(priority=LO)
        fence()
        wq_start(1, 0)
        x_copy(1, 0).start(priority=LO)
        x_copy(1, 1).start(priority=LO)
        fence()
        for gg in range(1, QA):
            for br in range(2):
                wq_start(br, gg)
        fence()
        issue(0, 0, 4)
        fence()
        issue(0, 4, B)
        acc[...] = jnp.zeros(acc.shape, f32)

        wq_wait(0, 0)
        for part in range(2):
            x_copy(0, part).wait()
            for j in range(4):
                qpiece(0, 0, j, part * B // 2, (part + 1) * B // 2)

        def qbody(i, carry):
            br, gg = i % 2, i // 2

            @pl.when(i == 1)
            def _():
                x_copy(1, 0).wait()
                x_copy(1, 1).wait()

            wq_wait(br, gg)

            @pl.when(i == 2)
            def _():
                issue(1, 0, 4)

            @pl.when(i == 4)
            def _():
                issue(1, 4, B)

            for j in range(4):
                qpiece(br, gg, j)
            return carry

        lax.fori_loop(1, 2 * QA, qbody, 0)

    kv = kv_v.at[g % 2]

    def rows_of(b):
        if isinstance(b, int):
            return pl.ds(b * SQ, SQ)
        return pl.ds(pl.multiple_of(b * SQ, 16), SQ)

    def tile(j):
        if isinstance(j, int):
            return pl.ds(j * 128, 128)
        return pl.ds(pl.multiple_of(j * 128, 128), 128)

    scores, probs = {}, {}

    def qk(c, b):
        if c == 'a':
            scores[c] = _qk(q_s[0, g, b], kv[b, 0])
        elif c == 'b0':
            scores[c] = _qk(q_s[1, g, b, :SQ], kv[b, 2])
        else:
            scores[c] = _qk(q_s[1, g, b, SQ:], kv[b, 3])

    def softmax(c):
        probs[c] = _softmax(scores.pop(c))

    def pv(c, b):
        if c not in probs:
            softmax(c)
        p, l = probs.pop(c)
        if c == 'a':
            oa = _pv(p, l, kv[b, 1])
            oa_s[rows_of(b), :DH] = oa[:SQ]
            oa_s[rows_of(b), DH:] = oa[SQ:]
        elif c == 'b0':
            ob_s[rows_of(b), :DH] = _pv(p, l, kv[b, 4])
        else:
            ob_s[rows_of(b), DH:] = _pv(p, l, kv[b, 5])

    def oproj(br, j, final=False):
        if isinstance(j, int) and j < 0:
            return
        t = lax.dot_general(wo_v[br, :, cols(g)], (oa_s, ob_s)[br][tile(j), :], NT, preferred_element_type=f32)
        t = acc[br * D:(br + 1) * D, tile(j)] + t
        if final:
            fin_s[br * D:(br + 1) * D, :] = t
        else:
            acc[br * D:(br + 1) * D, tile(j)] = t

    def finish(j):
        out_v[tile(j), :] = fin_s[...].T.astype(bf16)

    def wo_wait():
        for br in range(2):
            wo_copy(br, g).wait()

    def group(main):
        span = HALF if main else MID_SPAN
        NP = NPM if main else NPT
        per_point = EM if main else ET
        gn = g + 2

        @pl.when(gn < G)
        def _():
            for br in range(2):
                wo_copy(br, gn).start(priority=LO)

        if main:
            @pl.when(gn + QA < G)
            def _():
                wq_start(0, gn + QA)

        def wait_data(b):
            if main:
                kv_wait(g, b, HALF)
                wq_wait(b // HALF, g + QA)
            else:
                for bb in range(b, b + span):
                    kv_wait(g, bb, 1)
            if b == 0:
                wo_wait()

        def refill_b(b):
            @pl.when(jnp.logical_and(gn >= G - QA, gn < G))
            def _():
                kvb_start(gn, b)

            if main and b % 2 == 1:
                @pl.when(gn < G - QA)
                def _():
                    kvb_start(gn, b - 1, 2)

            if main and b == HALF - 1:
                @pl.when(gn + QA < G)
                def _():
                    wq_start(1, gn + QA)

        todo = []

        def emit_a(n):
            for _ in range(min(n, len(todo))):
                c, i = todo.pop(0)
                if main or c >= HALF:
                    kva_piece(g + c // B, c % B, i, NP)
                else:
                    @pl.when(g > G - QA)
                    def _():
                        kva_piece(g, c, i, NP)

        for b in range(B):
            if b % span == 0:
                with jax.named_scope('w%d' % b):
                    wait_data(b)
                todo.extend((c, i) for c in range(b + span, b + 2 * span) for i in range(2 * NP))
                if main:
                    qpiece(b // HALF, g + QA, b % HALF)
            emit_a(per_point)
            if b > 0:
                pv('b1', b - 1)
                emit_a(per_point)
            qk('a', b)
            emit_a(per_point)
            qk('b0', b)
            emit_a(per_point)
            pv('a', b)
            emit_a(per_point)
            qk('b1', b)
            emit_a(per_point)
            pv('b0', b)
            softmax('b1')
            if b % span == span - (2 if main else 1):
                emit_a(len(todo))
            if main and b % span != 0 and b < B - 1:
                qpiece(b // HALF, g + QA, b % HALF)
            oproj(0, b - 1)
            if b == B - 1 and not main:
                pv('b1', b)
            oproj(1, b - 2)
            if b >= 1:
                refill_b(b - 1)
        if main:
            pv('b1', B - 1)
            qpiece(1, g + QA, HALF - 1)
        oproj(1, B - 2)
        refill_b(B - 1)

    def last_group():
        def step(b, kind):
            with jax.named_scope('lw'):
                kv_wait(g, b, 1)
                if kind == 'first':
                    wo_wait()
            pieces = list(range(2 * NPT)) if kind == 'loop' else []

            def emit(n):
                for _ in range(min(n, len(pieces))):
                    kva_piece(G - 1, b + 1, pieces.pop(0), NPT)

            if kind == 'final':
                for j in range(NTILE - 2):
                    out_copy(j).start()
                fence()
                finish(NTILE - 2)
                out_copy(NTILE - 2).start()
            if kind == 'loop':
                emit(ET)
                finish(jnp.maximum(b - 2, 0))
            for c in ('a', 'b0', 'b1'):
                qk(c, b)
                emit(ET)
            for c in ('a', 'b0', 'b1'):
                pv(c, b)
                emit(ET if c != 'b1' else 2 * NPT)
            if kind == 'first':
                fin_s[...] = jnp.zeros(fin_s.shape, f32)
            else:
                oproj(0, b - 1, final=True)
                oproj(1, b - 1, final=True)

        step(0, 'first')

        def body(b, carry):
            step(b, 'loop')
            return carry

        lax.fori_loop(1, B - 1, body, 0)
        step(B - 1, 'final')
        finish(NTILE - 1)
        out_copy(NTILE - 1).start()
        with jax.named_scope('outwait'):
            for j in range(NTILE):
                out_copy(j).wait()

    @pl.when(g < G - QA)
    def _():
        with jax.named_scope('main'):
            group(main=True)

    @pl.when(jnp.logical_and(g >= G - QA, g < G - 1))
    def _():
        with jax.named_scope('mid'):
            group(main=False)

    @pl.when(g == G - 1)
    def _():
        with jax.named_scope('last'):
            last_group()


@jax.jit
def pallas_concat_heads__gqa_block_cached__mha_block_cached__near_ridge_kernel(
    A_x: jax.Array,
    A_k_cache: jax.Array,
    A_v_cache: jax.Array,
    A_wq: jax.Array,
    A_wo: jax.Array,
    B_x: jax.Array,
    B_k_cache: jax.Array,
    B_v_cache: jax.Array,
    B_wq: jax.Array,
    B_wo: jax.Array,
):
    hbm = pl.BlockSpec(memory_space=pltpu.MemorySpace.HBM)
    out = pl.pallas_call(
        _kernel,
        grid=(G,),
        in_specs=[hbm] * 10,
        out_specs=hbm,
        out_shape=jax.ShapeDtypeStruct((M, 2 * D), bf16),
        scratch_shapes=[
            pltpu.VMEM((2, M, D), bf16),
            pltpu.VMEM((2, D, H * DH), bf16),
            pltpu.VMEM((2, D, H * DH), bf16),
            pltpu.VMEM((2, B, 6, SK, DH), bf16),
            pltpu.VMEM((2, G, B, 2 * SQ, DH), bf16),
            pltpu.VMEM((M, GW), bf16),
            pltpu.VMEM((M, GW), bf16),
            pltpu.VMEM((2 * D, M), f32),
            pltpu.VMEM((2 * D, 128), f32),
            pltpu.VMEM((M, 2 * D), bf16),
            pltpu.SemaphoreType.DMA((2, 2)),
            pltpu.SemaphoreType.DMA((2, G)),
            pltpu.SemaphoreType.DMA((2, G)),
            pltpu.SemaphoreType.DMA((2, B)),
            pltpu.SemaphoreType.DMA((NTILE,)),
            pltpu.SemaphoreType.REGULAR,
        ],
        compiler_params=pltpu.CompilerParams(
            dimension_semantics=("arbitrary",),
            vmem_limit_bytes=100 * 1024 * 1024,
            disable_bounds_checks=True,
            disable_semaphore_checks=True,
        ),
    )(A_x.reshape(M, D), A_k_cache, A_v_cache, A_wq, A_wo.T,
      B_x.reshape(M, D), B_k_cache, B_v_cache, B_wq, B_wo.T)
    return out.reshape(B, SQ, 2 * D)
```

```python
import jax
import jax.numpy as jnp
from jax import lax
import jax.experimental.pallas as pl
import jax.experimental.pallas.tpu as pltpu

B, SQ, D = 8, 112, 448
H, SK, DH = 16, 512, 256
M = B * SQ
G = 8
GW = 2 * DH
HALF = B // 2
NTILE = M // 128
QSCALE = DH ** -0.5
NT = (((1,), (1,)), ((), ()))
bf16 = jnp.bfloat16
f32 = jnp.float32

QA = 3
NMAIN = G - QA
MID_SPAN = 2
HI, LO = 0, 1
NP_MAIN, NP_TAIL = 8, 4
EMIT_MAIN, EMIT_TAIL = 4, 2


def _qk(q, k):
    return lax.dot_general(q, k, NT, preferred_element_type=f32)


def _softmax(s):
    m = jnp.max(s, axis=-1, keepdims=True)
    p = jnp.exp(s - m)
    l = jnp.sum(p, axis=-1, keepdims=True)
    return p.astype(bf16), l


def _pv(p, l, v):
    o = jnp.dot(p, v, preferred_element_type=f32)
    r = pl.reciprocal(l, approx=True)
    r = r * (2.0 - l * r)
    return (o * r).astype(bf16)


def _kernel(xa_h, ka_h, va_h, wqa_h, woa_h, xb_h, kb_h, vb_h, wqb_h, wob_h, out_h,
            x_v, wq_v, wo_v, kv_v, q_s, oa_s, ob_s, acc, fin_s, out_v,
            x_sem, wq_sem, wo_sem, kv_sem, out_sem, fence_sem):
    g = pl.program_id(0)

    def cols(gg):
        return pl.ds(pl.multiple_of(gg * GW, GW), GW)

    def x_copy(br, part):
        rows = pl.ds(part * (M // 2), M // 2)
        return pltpu.make_async_copy((xa_h, xb_h)[br].at[rows], x_v.at[br, rows], x_sem.at[br, part])

    def wq_start(br, gg):
        pltpu.make_async_copy((wqa_h, wqb_h)[br].at[:, cols(gg)], wq_v.at[br, :, cols(gg)],
                              wq_sem.at[br, gg]).start(priority=LO)

    def wq_wait(br, gg):
        dst = wq_v.at[br, :, cols(gg)]
        pltpu.make_async_copy(dst, dst, wq_sem.at[br, gg]).wait()

    def wo_copy(br, gg):
        return pltpu.make_async_copy((woa_h, wob_h)[br].at[:, cols(gg)], wo_v.at[br, :, cols(gg)],
                                     wo_sem.at[br, gg])

    def chunk_sem(gg, b):
        if isinstance(gg, int):
            i = b // HALF * HALF if gg < NMAIN else b
        else:
            i = jnp.where(gg < NMAIN, b // HALF * HALF, b)
        return kv_sem.at[gg % 2, i]

    def kva_piece(gg, b, i, npiece):
        rows = pl.ds((i % npiece) * (SK // npiece), SK // npiece)
        src = (ka_h, va_h)[i // npiece]
        pltpu.make_async_copy(src.at[b, gg, rows], kv_v.at[gg % 2, b, i // npiece, rows],
                              chunk_sem(gg, b)).start(priority=HI)

    def kva_start(gg, b, n):
        dst, sem, bs = kv_v.at[gg % 2, pl.ds(b, n)], chunk_sem(gg, b), pl.ds(b, n)
        pltpu.make_async_copy(ka_h.at[bs, gg], dst.at[:, 0], sem).start(priority=LO)
        pltpu.make_async_copy(va_h.at[bs, gg], dst.at[:, 1], sem).start(priority=LO)

    def kvb_start(gg, b, n):
        dst, sem, bs = kv_v.at[gg % 2, pl.ds(b, n)], chunk_sem(gg, b), pl.ds(b, n)
        heads = pl.ds(2 * gg, 2)
        pltpu.make_async_copy(kb_h.at[bs, heads], dst.at[:, pl.ds(2, 2)], sem).start(priority=LO)
        pltpu.make_async_copy(vb_h.at[bs, heads], dst.at[:, pl.ds(4, 2)], sem).start(priority=LO)

    def kv_wait(b, n):
        dst = kv_v.at[g % 2, pl.ds(b, n)]
        pltpu.make_async_copy(dst, dst, kv_sem.at[g % 2, b]).wait()

    def out_copy(j):
        rows = pl.ds(j * 128, 128)
        return pltpu.make_async_copy(out_v.at[rows], out_h.at[rows], out_sem.at[j])

    def fence():
        pl.semaphore_signal(fence_sem, 1)
        pl.semaphore_wait(fence_sem, 1)

    kv = kv_v.at[g % 2]

    def rows_of(b):
        return pl.ds(b * SQ if isinstance(b, int) else pl.multiple_of(b * SQ, 16), SQ)

    def tile(j):
        return pl.ds(j * 128 if isinstance(j, int) else pl.multiple_of(j * 128, 128), 128)

    def qpiece(br, gg, j, b0=0, b1=B):
        c = pl.ds(pl.multiple_of(gg * GW + j * 128, 128), 128)
        q = jnp.dot(x_v[br, b0 * SQ:b1 * SQ], wq_v[br, :, c], preferred_element_type=f32)
        q = (q * QSCALE).astype(bf16)
        h, half = j // 2, j % 2
        for b in range(b0, b1):
            q_s[br, gg, b, h * SQ:(h + 1) * SQ, half * 128:(half + 1) * 128] = (
                q[(b - b0) * SQ:(b - b0 + 1) * SQ])

    scores, probs = {}, {}

    def qk(c, b):
        if c == 'a':
            scores[c] = _qk(q_s[0, g, b], kv[b, 0])
        elif c == 'b0':
            scores[c] = _qk(q_s[1, g, b, :SQ], kv[b, 2])
        else:
            scores[c] = _qk(q_s[1, g, b, SQ:], kv[b, 3])

    def softmax(c):
        probs[c] = _softmax(scores.pop(c))

    def pv(c, b):
        if c not in probs:
            softmax(c)
        p, l = probs.pop(c)
        if c == 'a':
            oa = _pv(p, l, kv[b, 1])
            oa_s[rows_of(b), :DH] = oa[:SQ]
            oa_s[rows_of(b), DH:] = oa[SQ:]
        elif c == 'b0':
            ob_s[rows_of(b), :DH] = _pv(p, l, kv[b, 4])
        else:
            ob_s[rows_of(b), DH:] = _pv(p, l, kv[b, 5])

    def oproj(br, j, final=False):
        if isinstance(j, int) and j < 0:
            return
        t = lax.dot_general(wo_v[br, :, cols(g)], (oa_s, ob_s)[br][tile(j), :], NT,
                            preferred_element_type=f32)
        t = acc[br * D:(br + 1) * D, tile(j)] + t
        if final:
            fin_s[br * D:(br + 1) * D, :] = t
        else:
            acc[br * D:(br + 1) * D, tile(j)] = t

    def finish(j):
        out_v[tile(j), :] = fin_s[...].T.astype(bf16)

    def wo_wait():
        for br in range(2):
            wo_copy(br, g).wait()

    @pl.when(g == 0)
    def _():
        def issue(gg, b):
            if b == 0:
                wo_copy(0, gg).start(priority=LO)
                wq_start(0, gg + QA)
                wo_copy(1, gg).start(priority=LO)
            else:
                wq_start(1, gg + QA)
            if gg == 0 and b == 0:
                kva_start(gg, b, HALF)
            kvb_start(gg, b, HALF)

        wq_start(0, 0)
        x_copy(0, 0).start(priority=LO)
        fence()
        x_copy(0, 1).start(priority=LO)
        fence()
        wq_start(1, 0)
        x_copy(1, 0).start(priority=LO)
        x_copy(1, 1).start(priority=LO)
        fence()
        for gg in range(1, QA):
            for br in range(2):
                wq_start(br, gg)
        fence()
        issue(0, 0)
        fence()
        issue(0, HALF)
        acc[...] = jnp.zeros(acc.shape, f32)

        wq_wait(0, 0)
        for part in range(2):
            x_copy(0, part).wait()
            for j in range(4):
                qpiece(0, 0, j, part * HALF, (part + 1) * HALF)

        def qbody(i, carry):
            br, gg = i % 2, i // 2

            @pl.when(i == 1)
            def _():
                x_copy(1, 0).wait()
                x_copy(1, 1).wait()

            wq_wait(br, gg)

            @pl.when(i == 2)
            def _():
                issue(1, 0)

            @pl.when(i == 4)
            def _():
                issue(1, HALF)

            for j in range(4):
                qpiece(br, gg, j)
            return carry

        lax.fori_loop(1, 2 * QA, qbody, 0)

    def group(main):
        span = HALF if main else MID_SPAN
        npiece = NP_MAIN if main else NP_TAIL
        emit_n = EMIT_MAIN if main else EMIT_TAIL
        gn = g + 2

        @pl.when(gn < G)
        def _():
            for br in range(2):
                wo_copy(br, gn).start(priority=LO)

        if main:
            @pl.when(gn + QA < G)
            def _():
                wq_start(0, gn + QA)

        def wait_data(b):
            if main:
                kv_wait(b, HALF)
                wq_wait(b // HALF, g + QA)
            else:
                for bb in range(b, b + span):
                    kv_wait(bb, 1)
            if b == 0:
                wo_wait()

        def refill_b(b):
            @pl.when(jnp.logical_and(gn >= NMAIN, gn < G))
            def _():
                kvb_start(gn, b, 1)

            if main and b % 2 == 1:
                @pl.when(gn < NMAIN)
                def _():
                    kvb_start(gn, b - 1, 2)

            if main and b == HALF - 1:
                @pl.when(gn + QA < G)
                def _():
                    wq_start(1, gn + QA)

        todo = []

        def emit(n):
            for _ in range(min(n, len(todo))):
                c, i = todo.pop(0)
                if main or c >= HALF:
                    kva_piece(g + c // B, c % B, i, npiece)
                else:
                    @pl.when(g > NMAIN)
                    def _():
                        kva_piece(g, c, i, npiece)

        for b in range(B):
            if b % span == 0:
                wait_data(b)
                todo.extend((c, i) for c in range(b + span, b + 2 * span) for i in range(2 * npiece))
                if main:
                    qpiece(b // HALF, g + QA, b % HALF)
            emit(emit_n)
            if b > 0:
                pv('b1', b - 1)
                emit(emit_n)
            qk('a', b)
            emit(emit_n)
            qk('b0', b)
            emit(emit_n)
            pv('a', b)
            emit(emit_n)
            qk('b1', b)
            emit(emit_n)
            pv('b0', b)
            softmax('b1')
            if b % span == span - (2 if main else 1):
                emit(len(todo))
            if main and b % span != 0 and b < B - 1:
                qpiece(b // HALF, g + QA, b % HALF)
            oproj(0, b - 1)
            if b == B - 1 and not main:
                pv('b1', b)
            oproj(1, b - 2)
            if b >= 1:
                refill_b(b - 1)
        if main:
            pv('b1', B - 1)
            qpiece(1, g + QA, HALF - 1)
        oproj(1, B - 2)
        refill_b(B - 1)

    def last_step(b, kind):
        kv_wait(b, 1)
        if kind == 'first':
            wo_wait()
        todo = list(range(2 * NP_TAIL)) if kind == 'loop' else []

        def emit(n):
            for _ in range(min(n, len(todo))):
                kva_piece(G - 1, b + 1, todo.pop(0), NP_TAIL)

        if kind == 'final':
            for j in range(NTILE - 2):
                out_copy(j).start()
            fence()
            finish(NTILE - 2)
            out_copy(NTILE - 2).start()
        if kind == 'loop':
            emit(EMIT_TAIL)
            finish(jnp.maximum(b - 2, 0))
        for c in ('a', 'b0', 'b1'):
            qk(c, b)
            emit(EMIT_TAIL)
        for c in ('a', 'b0', 'b1'):
            pv(c, b)
            emit(EMIT_TAIL if c != 'b1' else len(todo))
        if kind == 'first':
            fin_s[...] = jnp.zeros(fin_s.shape, f32)
        else:
            oproj(0, b - 1, final=True)
            oproj(1, b - 1, final=True)

    @pl.when(g < NMAIN)
    def _():
        group(main=True)

    @pl.when(jnp.logical_and(g >= NMAIN, g < G - 1))
    def _():
        group(main=False)

    @pl.when(g == G - 1)
    def _():
        last_step(0, 'first')

        def body(b, carry):
            last_step(b, 'loop')
            return carry

        lax.fori_loop(1, B - 1, body, 0)
        last_step(B - 1, 'final')
        finish(NTILE - 1)
        out_copy(NTILE - 1).start()
        for j in range(NTILE):
            out_copy(j).wait()


@jax.jit
def pallas_concat_heads__gqa_block_cached__mha_block_cached__near_ridge_kernel(
    A_x: jax.Array,
    A_k_cache: jax.Array,
    A_v_cache: jax.Array,
    A_wq: jax.Array,
    A_wo: jax.Array,
    B_x: jax.Array,
    B_k_cache: jax.Array,
    B_v_cache: jax.Array,
    B_wq: jax.Array,
    B_wo: jax.Array,
):
    hbm = pl.BlockSpec(memory_space=pltpu.MemorySpace.HBM)
    out = pl.pallas_call(
        _kernel,
        grid=(G,),
        in_specs=[hbm] * 10,
        out_specs=hbm,
        out_shape=jax.ShapeDtypeStruct((M, 2 * D), bf16),
        scratch_shapes=[
            pltpu.VMEM((2, M, D), bf16),
            pltpu.VMEM((2, D, H * DH), bf16),
            pltpu.VMEM((2, D, H * DH), bf16),
            pltpu.VMEM((2, B, 6, SK, DH), bf16),
            pltpu.VMEM((2, G, B, 2 * SQ, DH), bf16),
            pltpu.VMEM((M, GW), bf16),
            pltpu.VMEM((M, GW), bf16),
            pltpu.VMEM((2 * D, M), f32),
            pltpu.VMEM((2 * D, 128), f32),
            pltpu.VMEM((M, 2 * D), bf16),
            pltpu.SemaphoreType.DMA((2, 2)),
            pltpu.SemaphoreType.DMA((2, G)),
            pltpu.SemaphoreType.DMA((2, G)),
            pltpu.SemaphoreType.DMA((2, B)),
            pltpu.SemaphoreType.DMA((NTILE,)),
            pltpu.SemaphoreType.REGULAR,
        ],
        compiler_params=pltpu.CompilerParams(
            dimension_semantics=("arbitrary",),
            vmem_limit_bytes=100 * 1024 * 1024,
            disable_bounds_checks=True,
            disable_semaphore_checks=True,
        ),
    )(A_x.reshape(M, D), A_k_cache, A_v_cache, A_wq, A_wo.T,
      B_x.reshape(M, D), B_k_cache, B_v_cache, B_wq, B_wo.T)
    return out.reshape(B, SQ, 2 * D)
```

```python
import jax
import jax.numpy as jnp
from jax import lax
import jax.experimental.pallas as pl
import jax.experimental.pallas.tpu as pltpu

B, SQ, D = 8, 112, 448
H, SK, DH = 16, 512, 256
M = B * SQ
G = 8
GW = 2 * DH
HALF = B // 2
NTILE = M // 128
QSCALE = DH ** -0.5
NT = (((1,), (1,)), ((), ()))
bf16 = jnp.bfloat16
f32 = jnp.float32

QA = 3
NMAIN = G - QA
MID_SPAN = 2
HI, LO = 0, 1
NP_MAIN, NP_TAIL = 8, 4
EMIT_MAIN, EMIT_TAIL = 4, 2


def _qk(q, k):
    return lax.dot_general(q, k, NT, preferred_element_type=f32)


def _softmax(s):
    m = jnp.max(s, axis=-1, keepdims=True)
    p = jnp.exp(s - m)
    l = jnp.sum(p, axis=-1, keepdims=True)
    return p.astype(bf16), l


def _pv(p, l, v):
    o = jnp.dot(p, v, preferred_element_type=f32)
    r = pl.reciprocal(l, approx=True)
    r = r * (2.0 - l * r)
    return (o * r).astype(bf16)


def _kernel(xa_h, ka_h, va_h, wqa_h, woa_h, xb_h, kb_h, vb_h, wqb_h, wob_h, out_h,
            x_v, wq_v, wo_v, kv_v, q_s, oa_s, ob_s, acc, fin_s, out_v,
            x_sem, wq_sem, wo_sem, kv_sem, out_sem, fence_sem):
    g = pl.program_id(0)

    def cols(gg):
        return pl.ds(pl.multiple_of(gg * GW, GW), GW)

    def x_copy(br, part):
        rows = pl.ds(part * (M // 2), M // 2)
        return pltpu.make_async_copy((xa_h, xb_h)[br].at[rows], x_v.at[br, rows], x_sem.at[br, part])

    def wq_start(br, gg):
        pltpu.make_async_copy((wqa_h, wqb_h)[br].at[:, cols(gg)], wq_v.at[br, :, cols(gg)],
                              wq_sem.at[br, gg]).start(priority=LO)

    def wq_wait(br, gg):
        dst = wq_v.at[br, :, cols(gg)]
        pltpu.make_async_copy(dst, dst, wq_sem.at[br, gg]).wait()

    def wo_copy(br, gg):
        return pltpu.make_async_copy((woa_h, wob_h)[br].at[:, cols(gg)], wo_v.at[br, :, cols(gg)],
                                     wo_sem.at[br, gg])

    def chunk_sem(gg, b):
        if isinstance(gg, int):
            i = b // HALF * HALF if gg < NMAIN else b
        else:
            i = jnp.where(gg < NMAIN, b // HALF * HALF, b)
        return kv_sem.at[gg % 2, i]

    def kva_piece(gg, b, i, npiece):
        rows = pl.ds((i % npiece) * (SK // npiece), SK // npiece)
        src = (ka_h, va_h)[i // npiece]
        pltpu.make_async_copy(src.at[b, gg, rows], kv_v.at[gg % 2, b, i // npiece, rows],
                              chunk_sem(gg, b)).start(priority=HI)

    def kva_start(gg, b, n):
        dst, sem, bs = kv_v.at[gg % 2, pl.ds(b, n)], chunk_sem(gg, b), pl.ds(b, n)
        pltpu.make_async_copy(ka_h.at[bs, gg], dst.at[:, 0], sem).start(priority=LO)
        pltpu.make_async_copy(va_h.at[bs, gg], dst.at[:, 1], sem).start(priority=LO)

    def kvb_start(gg, b, n):
        dst, sem, bs = kv_v.at[gg % 2, pl.ds(b, n)], chunk_sem(gg, b), pl.ds(b, n)
        heads = pl.ds(2 * gg, 2)
        pltpu.make_async_copy(kb_h.at[bs, heads], dst.at[:, pl.ds(2, 2)], sem).start(priority=LO)
        pltpu.make_async_copy(vb_h.at[bs, heads], dst.at[:, pl.ds(4, 2)], sem).start(priority=LO)

    def kv_wait(b, n):
        dst = kv_v.at[g % 2, pl.ds(b, n)]
        pltpu.make_async_copy(dst, dst, kv_sem.at[g % 2, b]).wait()

    def out_copy(j):
        rows = pl.ds(j * 128, 128)
        return pltpu.make_async_copy(out_v.at[rows], out_h.at[rows], out_sem.at[j])

    def fence():
        pl.semaphore_signal(fence_sem, 1)
        pl.semaphore_wait(fence_sem, 1)

    kv = kv_v.at[g % 2]

    def rows_of(b):
        return pl.ds(b * SQ if isinstance(b, int) else pl.multiple_of(b * SQ, 16), SQ)

    def tile(j):
        return pl.ds(j * 128 if isinstance(j, int) else pl.multiple_of(j * 128, 128), 128)

    def qpiece(br, gg, j, b0=0, b1=B):
        c = pl.ds(pl.multiple_of(gg * GW + j * 128, 128), 128)
        q = jnp.dot(x_v[br, b0 * SQ:b1 * SQ], wq_v[br, :, c], preferred_element_type=f32)
        q = (q * QSCALE).astype(bf16)
        h, half = j // 2, j % 2
        for b in range(b0, b1):
            q_s[br, gg, b, h * SQ:(h + 1) * SQ, half * 128:(half + 1) * 128] = (
                q[(b - b0) * SQ:(b - b0 + 1) * SQ])

    scores, probs = {}, {}

    def qk(c, b):
        if c == 'a':
            scores[c] = _qk(q_s[0, g, b], kv[b, 0])
        elif c == 'b0':
            scores[c] = _qk(q_s[1, g, b, :SQ], kv[b, 2])
        else:
            scores[c] = _qk(q_s[1, g, b, SQ:], kv[b, 3])

    def softmax(c):
        probs[c] = _softmax(scores.pop(c))

    def pv(c, b):
        if c not in probs:
            softmax(c)
        p, l = probs.pop(c)
        if c == 'a':
            oa = _pv(p, l, kv[b, 1])
            oa_s[rows_of(b), :DH] = oa[:SQ]
            oa_s[rows_of(b), DH:] = oa[SQ:]
        elif c == 'b0':
            ob_s[rows_of(b), :DH] = _pv(p, l, kv[b, 4])
        else:
            ob_s[rows_of(b), DH:] = _pv(p, l, kv[b, 5])

    def oproj(br, j, final=False):
        if isinstance(j, int) and j < 0:
            return
        t = lax.dot_general(wo_v[br, :, cols(g)], (oa_s, ob_s)[br][tile(j), :], NT,
                            preferred_element_type=f32)
        t = acc[br * D:(br + 1) * D, tile(j)] + t
        if final:
            fin_s[br * D:(br + 1) * D, :] = t
        else:
            acc[br * D:(br + 1) * D, tile(j)] = t

    def finish(j):
        out_v[tile(j), :] = fin_s[...].T.astype(bf16)

    def wo_wait():
        for br in range(2):
            wo_copy(br, g).wait()

    @pl.when(g == 0)
    def _():
        def issue(gg, b):
            if b == 0:
                wo_copy(0, gg).start(priority=LO)
                wq_start(0, gg + QA)
                wo_copy(1, gg).start(priority=LO)
            else:
                wq_start(1, gg + QA)
            if gg == 0 and b == 0:
                kva_start(gg, b, HALF)
            kvb_start(gg, b, HALF)

        wq_start(0, 0)
        x_copy(0, 0).start(priority=LO)
        fence()
        x_copy(0, 1).start(priority=LO)
        fence()
        wq_start(1, 0)
        x_copy(1, 0).start(priority=LO)
        x_copy(1, 1).start(priority=LO)
        fence()
        for gg in range(1, QA):
            for br in range(2):
                wq_start(br, gg)
        fence()
        issue(0, 0)
        fence()
        issue(0, HALF)
        acc[...] = jnp.zeros(acc.shape, f32)

        wq_wait(0, 0)
        for part in range(2):
            x_copy(0, part).wait()
            for j in range(4):
                qpiece(0, 0, j, part * HALF, (part + 1) * HALF)

        def qbody(i, carry):
            br, gg = i % 2, i // 2

            @pl.when(i == 1)
            def _():
                x_copy(1, 0).wait()
                x_copy(1, 1).wait()

            wq_wait(br, gg)

            @pl.when(i == 2)
            def _():
                issue(1, 0)

            @pl.when(i == 4)
            def _():
                issue(1, HALF)

            for j in range(4):
                qpiece(br, gg, j)
            return carry

        lax.fori_loop(1, 2 * QA, qbody, 0)

    def group(main):
        span = HALF if main else MID_SPAN
        npiece = NP_MAIN if main else NP_TAIL
        emit_n = EMIT_MAIN if main else EMIT_TAIL
        gn = g + 2

        def wait_data(b):
            if main:
                kv_wait(b, HALF)
                wq_wait(b // HALF, g + QA)
            else:
                for bb in range(b, b + span):
                    kv_wait(bb, 1)
            if b == 0:
                wo_wait()

                @pl.when(gn < G)
                def _():
                    for br in range(2):
                        wo_copy(br, gn).start(priority=LO)

                if main:
                    @pl.when(gn + QA < G)
                    def _():
                        wq_start(0, gn + QA)

        def refill_b(b):
            @pl.when(jnp.logical_and(gn >= NMAIN, gn < G))
            def _():
                kvb_start(gn, b, 1)

            if main and b % 2 == 1:
                @pl.when(gn < NMAIN)
                def _():
                    kvb_start(gn, b - 1, 2)

            if main and b == HALF - 1:
                @pl.when(gn + QA < G)
                def _():
                    wq_start(1, gn + QA)

        todo = []

        def emit(n):
            for _ in range(min(n, len(todo))):
                c, i = todo.pop(0)
                if main or c >= HALF:
                    kva_piece(g + c // B, c % B, i, npiece)
                else:
                    @pl.when(g > NMAIN)
                    def _():
                        kva_piece(g, c, i, npiece)

        for b in range(B):
            if b % span == 0:
                wait_data(b)
                todo.extend((c, i) for c in range(b + span, b + 2 * span) for i in range(2 * npiece))
                if main:
                    qpiece(b // HALF, g + QA, b % HALF)
            emit(emit_n)
            if b > 0:
                pv('b1', b - 1)
                emit(emit_n)
            qk('a', b)
            emit(emit_n)
            qk('b0', b)
            emit(emit_n)
            pv('a', b)
            emit(emit_n)
            qk('b1', b)
            emit(emit_n)
            pv('b0', b)
            softmax('b1')
            if b % span == span - (2 if main else 1):
                emit(len(todo))
            if main and b % span != 0 and b < B - 1:
                qpiece(b // HALF, g + QA, b % HALF)
            oproj(0, b - 1)
            if b == B - 1 and not main:
                pv('b1', b)
            oproj(1, b - 2)
            if b >= 1:
                refill_b(b - 1)
        if main:
            pv('b1', B - 1)
            qpiece(1, g + QA, HALF - 1)
        oproj(1, B - 2)
        refill_b(B - 1)

    def last_step(b, kind):
        kv_wait(b, 1)
        if kind == 'first':
            wo_wait()
        todo = list(range(2 * NP_TAIL)) if kind == 'loop' else []

        def emit(n):
            for _ in range(min(n, len(todo))):
                kva_piece(G - 1, b + 1, todo.pop(0), NP_TAIL)

        if kind == 'final':
            for j in range(NTILE - 2):
                out_copy(j).start()
            fence()
            finish(NTILE - 2)
            out_copy(NTILE - 2).start()
        if kind == 'loop':
            emit(EMIT_TAIL)
            finish(jnp.maximum(b - 2, 0))
        for c in ('a', 'b0', 'b1'):
            qk(c, b)
            emit(EMIT_TAIL)
        for c in ('a', 'b0', 'b1'):
            pv(c, b)
            emit(EMIT_TAIL if c != 'b1' else len(todo))
        if kind == 'first':
            fin_s[...] = jnp.zeros(fin_s.shape, f32)
        else:
            oproj(0, b - 1, final=True)
            oproj(1, b - 1, final=True)

    @pl.when(g < NMAIN)
    def _():
        group(main=True)

    @pl.when(jnp.logical_and(g >= NMAIN, g < G - 1))
    def _():
        group(main=False)

    @pl.when(g == G - 1)
    def _():
        last_step(0, 'first')

        def body(b, carry):
            last_step(b, 'loop')
            return carry

        lax.fori_loop(1, B - 1, body, 0)
        last_step(B - 1, 'final')
        finish(NTILE - 1)
        out_copy(NTILE - 1).start()
        for j in range(NTILE):
            out_copy(j).wait()


@jax.jit
def pallas_concat_heads__gqa_block_cached__mha_block_cached__near_ridge_kernel(
    A_x: jax.Array,
    A_k_cache: jax.Array,
    A_v_cache: jax.Array,
    A_wq: jax.Array,
    A_wo: jax.Array,
    B_x: jax.Array,
    B_k_cache: jax.Array,
    B_v_cache: jax.Array,
    B_wq: jax.Array,
    B_wo: jax.Array,
):
    hbm = pl.BlockSpec(memory_space=pltpu.MemorySpace.HBM)
    out = pl.pallas_call(
        _kernel,
        grid=(G,),
        in_specs=[hbm] * 10,
        out_specs=hbm,
        out_shape=jax.ShapeDtypeStruct((M, 2 * D), bf16),
        scratch_shapes=[
            pltpu.VMEM((2, M, D), bf16),
            pltpu.VMEM((2, D, H * DH), bf16),
            pltpu.VMEM((2, D, H * DH), bf16),
            pltpu.VMEM((2, B, 6, SK, DH), bf16),
            pltpu.VMEM((2, G, B, 2 * SQ, DH), bf16),
            pltpu.VMEM((M, GW), bf16),
            pltpu.VMEM((M, GW), bf16),
            pltpu.VMEM((2 * D, M), f32),
            pltpu.VMEM((2 * D, 128), f32),
            pltpu.VMEM((M, 2 * D), bf16),
            pltpu.SemaphoreType.DMA((2, 2)),
            pltpu.SemaphoreType.DMA((2, G)),
            pltpu.SemaphoreType.DMA((2, G)),
            pltpu.SemaphoreType.DMA((2, B)),
            pltpu.SemaphoreType.DMA((NTILE,)),
            pltpu.SemaphoreType.REGULAR,
        ],
        compiler_params=pltpu.CompilerParams(
            dimension_semantics=("arbitrary",),
            vmem_limit_bytes=100 * 1024 * 1024,
            disable_bounds_checks=True,
            disable_semaphore_checks=True,
        ),
    )(A_x.reshape(M, D), A_k_cache, A_v_cache, A_wq, A_wo.T,
      B_x.reshape(M, D), B_k_cache, B_v_cache, B_wq, B_wo.T)
    return out.reshape(B, SQ, 2 * D)
```
